```python
import os as _os
_os.environ.setdefault("JAX_PLATFORMS", "cpu")
import jax
import jax.numpy as jnp

def _softmax(x, axis=-1):
    return jax.nn.softmax(x, axis=axis)
def _gelu(x):
    return jax.nn.gelu(x, approximate=True)
def _silu(x):
    return jax.nn.silu(x)
def _sigmoid(x):
    return jax.nn.sigmoid(x)
def _layernorm(x, axis=-1, eps=1e-5):
    m = jnp.mean(x, axis=axis, keepdims=True)
    v = jnp.var(x, axis=axis, keepdims=True)
    return (x - m) / jnp.sqrt(v + eps)
def _scatter_add(tgt, idx, src, axis=0):
    return tgt.at[idx].add(src)
def _segment_sum(src, seg, n):
    return jax.ops.segment_sum(src, seg, n)
class _Rng:
    def __init__(self, key):
        self._k = key
    def _next(self):
        self._k, sub = jax.random.split(self._k)
        return sub
    def normal(self, shape):
        return jax.random.normal(self._next(), shape, dtype=jnp.bfloat16)
    def randint(self, lo, hi, shape):
        return jax.random.randint(self._next(), shape, lo, hi, dtype=jnp.int32)
    def uniform(self, shape, lo=0.0, hi=1.0):
        return jax.random.uniform(self._next(), shape, jnp.bfloat16, lo, hi)
    def permutation(self, n):
        return jax.random.permutation(self._next(), n)


kernel_name = 'gated_mix__ssm_conv_h3__mixer_s_mlp__prompt'

def setup_inputs():
    _rng = _Rng(jax.random.key(int.from_bytes(__import__("os").urandom(4), "little")))
    _w = (lambda a: (lambda t: t.astype(jnp.bfloat16) if jnp.issubdtype(t.dtype, jnp.floating) else t)(jnp.asarray(a)))
    def _A_setup():
        B, S, D = 1, 2048, 576
        ks = 4
        return {
            "q": _w((lambda *s: _rng.normal(s) * 0.05)(B, S, D)),
            "k": _w((lambda *s: _rng.normal(s) * 0.4)(B, S, D)),
            "v": _w((lambda *s: _rng.normal(s) * 0.4)(B, S, D)),
            "shift_k": _w((lambda *s: _rng.normal(s) * 0.4)(D, ks) * 0.5),
            "ssm_k": _w((lambda *s: _rng.normal(s) * 0.4)(D, S) * (1.0 / S ** 0.5)),
            "ssm_D": _w((lambda *s: _rng.normal(s) * 0.4)(D)),
        }
    _A_in = _A_setup()

    def _B_setup():
        B, S, D, F = 1, 2048, 576, 4608
        return {
            "x":  _w((lambda *s: _rng.normal(s) * 0.05)(B, S, D)),
            "w1": _w((lambda *s: _rng.normal(s) * 0.2)(D, D) * (D ** -0.5)),
            "w2": _w((lambda *s: _rng.normal(s) * 0.2)(D, D) * (D ** -0.5)),
            "w3": _w((lambda *s: _rng.normal(s) * 0.2)(D, F) * (D ** -0.5)),
            "w4": _w((lambda *s: _rng.normal(s) * 0.2)(F, D) * (F ** -0.5)),
        }
    _B_in = _B_setup()

    return {
        "A_q": _A_in["q"],
        "A_k": _A_in["k"],
        "A_v": _A_in["v"],
        "A_shift_k": _A_in["shift_k"],
        "A_ssm_k": _A_in["ssm_k"],
        "A_ssm_D": _A_in["ssm_D"],
        "B_x": _B_in["x"],
        "B_w1": _B_in["w1"],
        "B_w2": _B_in["w2"],
        "B_w3": _B_in["w3"],
        "B_w4": _B_in["w4"],
        "gate_w": _w((lambda *s: _rng.normal(s) * 0.05)(576) * 16.0),
    }

def reference(A_q, A_k, A_v, A_shift_k, A_ssm_k, A_ssm_D, B_x, B_w1, B_w2, B_w3, B_w4, gate_w):
    def _A_ref(q, k, v, shift_k, ssm_k, ssm_D):
        B, S, D = q.shape
        ks = shift_k.shape[-1]
        k_pad = jnp.pad(k, ((0, 0), (ks - 1, 0), (0, 0)))
        k_shift = jnp.zeros_like(k)
        for t in range(ks):
            k_shift = k_shift + k_pad[:, t:t + S, :] * shift_k[:, ks - 1 - t][None, None, :]
        kv = k_shift * v
        L = 2 * S
        kv_pad = jnp.pad(kv, ((0, 0), (0, S), (0, 0)))
        kf_pad = jnp.pad(ssm_k, ((0, 0), (0, S)))
        kv_f = (lambda x, axes=(-2,-1): jnp.fft.rfft2(x.astype(jnp.float32), axes=axes))(kv_pad[:, None, :, :], axes=(1, 2))
        kf_f = (lambda x, axes=(-2,-1): jnp.fft.rfft2(x.astype(jnp.float32), axes=axes))(kf_pad[:, None, :], axes=(1, 2))
        kf_f = (lambda x, *d: x.transpose(*d))(kf_f, 1, 2, 0)
        y_f = kv_f * kf_f[None, :, :, :]
        y = (lambda x, s, axes=(-2,-1): jnp.fft.irfft2(x, s=s, axes=axes).astype(jnp.bfloat16))(y_f, (1, L), axes=(1, 2))[:, 0, :S, :]
        y = y + kv * ssm_D[None, None, :]
        return q * y

    def _B_ref(x, w1, w2, w3, w4):
        B, S, D = x.shape
        h = _gelu(_layernorm(x, axis=-1) @ w1)
        c = D // 4
        g0 = jnp.pad(h[:, :, 0*c:1*c], ((0, 0), (1, 0), (0, 0)))[:, :S, :]
        g1 = jnp.pad(h[:, :, 1*c:2*c], ((0, 0), (0, 1), (0, 0)))[:, 1:, :]
        g2 = jnp.pad(h[:, :, 2*c:3*c], ((0, 0), (2, 0), (0, 0)))[:, :S, :]
        g3 = jnp.pad(h[:, :, 3*c:   ], ((0, 0), (0, 2), (0, 0)))[:, 2:, :]
        hs = jnp.concatenate([g0, g1, g2, g3], axis=-1) @ w2
        x1 = x + hs
        h2 = _gelu(_layernorm(x1, axis=-1) @ w3) @ w4
        return x1 + h2

    x = A_q
    g = _sigmoid((x * gate_w).sum(-1, keepdims=True))
    a = _A_ref(x, A_k, A_v, A_shift_k, A_ssm_k, A_ssm_D)
    b = _B_ref(x, B_w1, B_w2, B_w3, B_w4)
    return g * a + (1 - g) * b
```

```python
import math
import numpy as np
import jax
import jax.numpy as jnp
from jax import lax
import jax.experimental.pallas as pl
import jax.experimental.pallas.tpu as pltpu

S, D, F = 2048, 576, 4608
CH = 128
NCH = S // CH
f32, bf16, u32 = jnp.float32, jnp.bfloat16, jnp.uint32

T = 512
NT = S // T
FC = 512
NF = F // FC
CS = D // NF
TIES = 9
CB, CI = 32, 32
ORDER = (1, 4, 0, 2, 5, 3, 6)
MP = D // 4

_C0 = math.sqrt(2.0 / math.pi)
GS = (_C0 * 0.044715) ** (1.0 / 3.0)
GK = _C0 / GS
KAPPA = 0.5 / GS

SA = [{(0, 0): 1, (1, 1): 1}, {(1, 0): 1, (1, 1): 1}, {(0, 0): 1}, {(1, 1): 1},
      {(0, 0): 1, (0, 1): 1}, {(1, 0): 1, (0, 0): -1}, {(0, 1): 1, (1, 1): -1}]
SB = [{(0, 0): 1, (1, 1): 1}, {(0, 0): 1}, {(0, 1): 1, (1, 1): -1}, {(1, 0): 1, (0, 0): -1},
      {(1, 1): 1}, {(0, 0): 1, (0, 1): 1}, {(1, 0): 1, (1, 1): 1}]
SC = np.array([[1, 0, 0, 1], [0, 0, 1, -1], [0, 1, 0, 1], [1, 0, 1, 0], [-1, 1, 0, 0], [0, 0, 0, 1], [1, 0, 0, 0]])


def _single(ps):
    inv = np.rint(np.linalg.inv(SC[list(ps)].astype(np.float64))).astype(int)
    out = {}
    for n, p in enumerate(ps):
        lam = inv[:, n].reshape(2, 2)
        i0, j0 = np.argwhere(lam != 0)[0]
        a, b = lam[:, j0] * lam[i0, j0], lam[i0, :].copy()
        assert (np.outer(a, b) == lam).all()
        if (b <= 0).all():
            a, b = -a, -b
        out[p] = ({i: int(a[i]) for i in range(2) if a[i]}, {j: int(b[j]) for j in range(2) if b[j]})
    return out


_PLAN = {9: (3, [(1, 3, 2, 5), (2, 4, 3, 6), (0, 3, 2, 5)]), 4: (2, []),
         6: (2, [(0, 1, 2, 5), (0, 1, 2, 5)]), 5: (1, [(1, 3, 2, 5), (2, 4, 1, 5), (0, 1, 2, 5)])}


def _level(depth):
    n_pairs, singles = _PLAN[depth]
    terms = [[] for _ in range(7)]
    for t in range(n_pairs):
        kk = (2 * t, 2 * t + 1)
        for p in range(7):
            terms[p].append(({(i, kk[k]): c for (i, k), c in SA[p].items()},
                             {(j, kk[k]): c for (k, j), c in SB[p].items()}))
    for n, ps in enumerate(singles):
        kb = 2 * n_pairs + n
        for p, (a, b) in _single(ps).items():
            terms[p].append(({(i, kb): c for i, c in a.items()}, {(j, kb): c for j, c in b.items()}))
    return terms


def _lin(items):
    acc = None
    for c, v in sorted(items, key=lambda cv: -cv[0]):
        if acc is None:
            acc = v if c > 0 else -v
        else:
            acc = acc + v if c > 0 else acc - v
    return acc


def _deep_operands(blocks, side, levels):
    if levels == 0:
        return [[b[0] for b in blocks]]
    h = len(blocks[0]) // 2
    out = []
    for terms in _level(len(blocks)):
        nxt = [[_lin([(c, blocks[kb][i * h + s]) for (i, kb), c in t[side].items()]) for s in range(h)]
               for t in terms]
        out += _deep_operands(nxt, side, levels - 1)
    return out


def _deep_group(get, side, p1):
    terms = _level(9)[p1]
    nxt = [[_lin([(c, get(kb, i * 2 + s)) for (i, kb), c in t[side].items()]) for s in range(2)] for t in terms]
    return _deep_operands(nxt, side, 1)


_UP_ORDER = (1, 3, 2, 4, 0, 5, 6)


def _combine7(p):
    return [(p[3] - p[4]) + p[0] + p[6], p[2] + p[4], p[1] + p[3], (p[2] - p[1]) + p[0] + p[5]]


def _combine_top(get):
    res = [[None] * 4 for _ in range(4)]
    for p1 in range(7):
        for q2 in range(4):
            v = get(p1, q2)
            for q in range(4):
                c = SC[p1, q]
                if c:
                    i, j = (q // 2) * 2 + q2 // 2, (q % 2) * 2 + q2 % 2
                    res[i][j] = v if res[i][j] is None else (res[i][j] + v if c > 0 else res[i][j] - v)
    return res


def _square_operands(blk, table):
    if len(blk) == 1:
        return [blk[0][0]]
    h = len(blk) // 2
    out = []
    for p in range(7):
        nxt = [[_lin([(c, blk[i * h + r][j * h + s]) for (i, j), c in table[p].items()]) for s in range(h)]
               for r in range(h)]
        out += _square_operands(nxt, table)
    return out


def _combine(get, levels, base=0):
    if levels == 0:
        return [[get(base)]]
    n, h = 7 ** (levels - 1), 2 ** (levels - 1)
    res = [[None] * (2 * h) for _ in range(2 * h)]
    for p in range(7):
        sub = _combine(get, levels - 1, base + p * n)
        for q in range(4):
            c = SC[p, q]
            if c == 0:
                continue
            for r in range(h):
                for s in range(h):
                    i, j = (q // 2) * h + r, (q % 2) * h + s
                    cur = res[i][j]
                    res[i][j] = sub[r][s] if cur is None else (cur + sub[r][s] if c > 0 else cur - sub[r][s])
    return res


DEPTH = [len(t2) for t1 in _level(9) for t2 in _level(len(t1))]
NPROD = len(DEPTH)
TILE0 = [sum((d + 1) // 2 for d in DEPTH[:p]) for p in range(NPROD + 1)]
NTILE = TILE0[-1]


def _pack(v):
    return pltpu.bitcast(v.astype(bf16), u32)


def _unpack(v):
    return pltpu.bitcast(v, bf16)


def _rows2(w):
    return [pltpu.unpack_elementwise(w, index=i, packed_dtype=bf16, unpacked_dtype=f32) for i in range(2)]


def _join2(even, odd):
    return pltpu.pack_elementwise([even, odd], packed_dtype=bf16)


def _gelu_u(u):
    return u + u * jnp.tanh(u * (u * u + GK))


def _ln(x, scale):
    m = jnp.sum(x, axis=0, keepdims=True) * (1.0 / D)
    xc = x - m
    v = jnp.sum(xc * xc, axis=0, keepdims=True) * (1.0 / D)
    return xc * (lax.rsqrt(v + 1e-5) * scale)


def _col(row):
    b = jnp.broadcast_to(row, (128, D))
    b = jnp.concatenate([b, jnp.zeros((128, 64), f32)], axis=1)
    return b.T[:D, :]


def _shift_lanes(x, n):
    size = x.shape[1]
    r = pltpu.roll(x, n % size, 1)
    lane = lax.broadcasted_iota(jnp.int32, (x.shape[0], 128), 1)
    if n > 0:
        edge = jnp.where(lane >= n, r[:, :128], jnp.zeros_like(r[:, :128]))
        return jnp.concatenate([edge, r[:, 128:]], axis=1)
    edge = jnp.where(lane < 128 + n, r[:, -128:], jnp.zeros_like(r[:, -128:]))
    return jnp.concatenate([r[:, :-128], edge], axis=1)


def _toeplitz(k, u):
    ys = []
    for a in range(len(u)):
        y = k[0] * u[a]
        for j in range(1, a + 1):
            y = y + k[j] * u[a - j]
        ys.append(y)
    return ys


def _transform_tables():
    def words(x):
        bits = x.astype(bf16).view(np.uint16).astype(np.uint32)
        return bits[:, 0::2] | (bits[:, 1::2] << 16)
    f, lane, m = np.ogrid[:4, :CH, :CH]
    angle = ((4 * m + 1) * (4 * ((lane - 32 * f) % CH) + f) % 2048) * (np.pi / 1024.0)
    fwd = np.concatenate([np.cos(angle), np.sin(angle)], axis=2)
    return words(fwd), words(fwd.transpose(0, 2, 1) / T)


def _kernel(zero_ref, q_hbm, k_hbm, v_hbm, sk_ref, ssmk_hbm, ssmd_ref, w1_hbm, w2_hbm, w3_hbm, w4_hbm, gw_ref, f_hbm, g_hbm,
            out_hbm,
            q_v, k_v, v_v, ssmk_v, w1_v, w2_v, w3_v, w4_v, w1t, w2t, cols, fmat, gmat,
            h_v, g_v, x1_v, ga_v, o_v, xa, wb, wa, acc0, acc1, acc2, acc3, zb0, zb1, zb2, zb3, xn0, xn1, pb0, pb1, pb2, pb3,
            sem_q, sem_w, sem_c, sem_f, sem_out):
    pb = (pb0, pb1, pb2, pb3)
    xnb = (xn0, xn1)
    zbs = (zb0, zb1, zb2, zb3)
    acc = (acc0, acc1, acc2, acc3)
    cp_q = [pltpu.make_async_copy(q_hbm.at[:, pl.ds(b * T, T)], q_v.at[b], sem_q.at[b]) for b in range(NT)]
    cp_w1 = pltpu.make_async_copy(w1_hbm, w1_v, sem_w.at[0])
    cp_w2 = pltpu.make_async_copy(w2_hbm, w2_v, sem_w.at[1])
    cp_out = [pltpu.make_async_copy(o_v.at[b], out_hbm.at[:, pl.ds(b * T, T)], sem_out.at[b]) for b in range(NT)]

    def cp_mlp(i):
        c = pl.ds(pl.multiple_of(i * FC, FC), FC)
        return [pltpu.make_async_copy(src.bitcast(u32).at[:, c], dst.at[i], sem_f.at[n, i])
                for n, (src, dst) in enumerate(((w3_hbm, w3_v), (w4_hbm, w4_v)))]

    def cp_conv(i):
        words = pl.ds(pl.multiple_of(i * (CS // 2), CS // 2), CS // 2)
        return [pltpu.make_async_copy(src.bitcast(u32).at[words, :], dst.at[i], sem_c.at[n, i])
                for n, (src, dst) in enumerate(((k_hbm, k_v), (v_hbm, v_v), (ssmk_hbm, ssmk_v)))]

    def zero(n):
        return pl.multiple_of(zero_ref[n], 64)

    def schedule(pieces, slots):
        total, now, out = sum(w for w, _ in pieces), 0, [[] for _ in range(slots)]
        for w, fn in pieces:
            out[min(slots - 1, int((now + w / 2) * slots / total))].append(fn)
            now += w
        return out

    def both(*plans):
        return [[fn for part in slot for fn in part] for slot in zip(*plans, strict=True)]

    def tied(w, *due):
        step = w.shape[0] // 8 // len(due) * 8
        parts = []
        for j, fns in enumerate(due):
            tie = None
            for fn in fns:
                t = fn()
                if t is not None:
                    t = pltpu.bitcast(t, u32)
                    tie = t if tie is None else tie | t
            top = w[j * step:j * step + 8]
            if tie is not None:
                left = top[:, :128] | (tie & jnp.full((8, 128), zero_ref[0], jnp.int32).astype(u32))
                top = jnp.concatenate([left, top[:, 128:]], axis=1) if w.shape[1] > 128 else left
            parts += [top, w[j * step + 8:(j + 1) * step if j + 1 < len(due) else w.shape[0]]]
        return jnp.concatenate(parts, axis=0)

    def token(w):
        t = w[:8, :128]
        for r in range(8, w.shape[0], 8):
            t = t | w[r:r + 8, :128]
        return t

    def transposed(w):
        w = w.astype(f32)
        w = jnp.concatenate([w, jnp.zeros((D, 64), f32)], axis=1)
        w = jnp.concatenate([w, jnp.zeros((64, D + 64), f32)], axis=0)
        return pltpu.bitcast(w.astype(bf16).T, u32)[:D // 2, :]

    def moments(state, x):
        if not state:
            state.update(pivot=jnp.broadcast_to(x[:1], (8, 128)), s1=None, s2=None)
        for r in range(0, x.shape[0], 8):
            d = x[r:r + 8] - state['pivot']
            state['s1'] = d if state['s1'] is None else state['s1'] + d
            state['s2'] = d * d if state['s2'] is None else state['s2'] + d * d

    def mean_scale(state):
        m = jnp.sum(state['s1'], axis=0, keepdims=True) * (1.0 / D)
        v = jnp.sum(state['s2'], axis=0, keepdims=True) * (1.0 / D) - m * m
        state['mean'] = state['pivot'] + m
        state['scale'] = jnp.broadcast_to(lax.rsqrt(jnp.maximum(v, 0.0) + 1e-5) * GS, (8, 128))
        return state['scale']

    def normalized(state, x):
        return jnp.concatenate([(x[r:r + 8] - state['mean']) * state['scale'] for r in range(0, x.shape[0], 8)], axis=0)

    stats = [{} for _ in range(S // 128)]

    def stats1(n):
        b, s = divmod(n, 4)
        gate = []

        def piece(r):
            x = q_v[b + zero(0), r:r + 48, s * 128:(s + 1) * 128].astype(f32)
            moments(stats[n], x)
            xw = x * cols[5, r:r + 48, :]
            for j in range(0, 48, 8):
                gate[:] = [xw[j:j + 8] + gate[0] if gate else xw[j:j + 8]]
            if r + 48 < D:
                return stats[n]['s2'] + gate[0]
            g = jnp.broadcast_to(jax.nn.sigmoid(jnp.sum(gate[0], axis=0, keepdims=True)), (8, 128))
            g_v[:, n * 128:(n + 1) * 128] = g
            return mean_scale(stats[n]) + g
        return [(42, lambda r=r: piece(r)) for r in range(0, D, 48)]

    def stage1(n, due):
        b, s = divmod(n, 4)
        w = _unpack(tied(w1t[zero(0)], *due))[:, :D]
        x = normalized(stats[n], q_v[b + zero(1), :, s * 128:(s + 1) * 128].astype(f32))
        z = jnp.dot(w, x.astype(bf16), preferred_element_type=f32)

        def act(r):
            h = _gelu_u(z[r:r + 48])
            h_v[r:r + 48, n * 128:(n + 1) * 128] = h
            return token(pltpu.bitcast(h, u32))
        return [(36, lambda r=r: act(r)) for r in range(0, D, 48)], []

    def stage2(n, due):
        grp = D // 4
        b, s = divmod(n, 4)
        c0 = n * 128
        w = _unpack(tied(w2t[zero(0)], *due))[:, :D]
        parts = []
        for gi, k in enumerate((1, -1, 2, -2)):
            rows = slice(gi * grp, (gi + 1) * grp)
            cur = h_v[rows, c0:c0 + 128]
            if k > 0:
                halo = h_v[rows, c0 - 128:c0] if c0 > 0 else jnp.zeros((grp, 128), f32)
                parts.append(pltpu.roll(jnp.concatenate([halo, cur], axis=1), k, 1)[:, 128:])
            else:
                halo = h_v[rows, c0 + 128:c0 + 256] if c0 + 128 < S else jnp.zeros((grp, 128), f32)
                parts.append(pltpu.roll(jnp.concatenate([cur, halo], axis=1), 256 + k, 1)[:, :128])
        z = jnp.dot(w, jnp.concatenate(parts, axis=0).astype(bf16), preferred_element_type=f32)
        c = slice(s * 128, (s + 1) * 128)
        state = {}

        def residual(r):
            x1 = q_v[b + zero(2), r:r + 48, c].astype(f32) + KAPPA * z[r:r + 48]
            x1_v[b, r:r + 48, c] = x1
            moments(state, x1)
            return state['s2'] if r + 48 < D else mean_scale(state)

        def norm(r):
            xn = normalized(state, x1_v[b + zero(0), r:r + 48, c])
            xnb[b % 2][r:r + 48, c] = xn
            return token(pltpu.bitcast(xn, u32))
        return ([(40, lambda r=r: residual(r)) for r in range(0, D, 48)],
                [(18, lambda r=r: norm(r)) for r in range(0, D, 48)])

    def clear(j):
        t, p = divmod(j, NPROD)
        acc[t][p * MP:(p + 1) * MP, :] = jnp.zeros((MP, 128), f32)
        return acc[t][pl.ds(zero(0), 8), :]

    def x_operands(b):
        groups = {}

        def piece(p, n):
            p1, p2 = divmod(p, 7)
            if p1 not in groups:
                get = lambda kb, s: xnb[b % 2][pl.ds(zero(8 + p1) + kb * 64, 64), s * 128:(s + 1) * 128]
                groups[p1] = _deep_group(get, 0, p1)
            pair = groups[p1][p2][2 * n:2 * n + 2]
            if len(pair) == 1:
                pair = pair + [jnp.zeros((64, 128), f32)]
            w = pltpu.bitcast(jnp.concatenate(pair, axis=0).astype(bf16).T, u32)
            xa[b, TILE0[p] + n] = w
            return w[56:]

        return [(33, lambda p=p, n=n: piece(p, n)) for p in range(NPROD) for n in range(TILE0[p + 1] - TILE0[p])]

    def w3_operands(i, p1):
        ii = i + zero(8 + p1)
        words = lambda kb, s: _rows2(w3_v[ii, kb * 32:(kb + 1) * 32, s * 128:(s + 1) * 128])
        ops = [_deep_group(lambda kb, s: words(kb, s)[h], 1, p1) for h in range(2)]
        for p2 in range(7):
            for n in range(DEPTH[p1 * 7 + p2]):
                wb[TILE0[p1 * 7 + p2] + n // 2, (n % 2) * 32:(n % 2) * 32 + 32, :] = _join2(ops[0][p2][n], ops[1][p2][n])

    def w4_operands(i):
        mid = {}

        def middle(p1, r, s):
            if (p1, r, s) not in mid:
                ii = i + zero(8 + p1)
                words = [(c, _rows2(w4_v[ii, (2 * m + r) * 72:(2 * m + r + 1) * 72,
                                         (2 * k + s) * 128:(2 * k + s + 1) * 128]))
                         for (m, k), c in SA[p1].items()]
                mid[p1, r, s] = [_lin([(c, w[h]) for c, w in words]) for h in range(2)]
            return mid[p1, r, s]

        def piece(p1, p2):
            w = _join2(*[_lin([(c, middle(p1, r, s)[h]) for (r, s), c in SA[p2].items()]) for h in range(2)])
            wa[(p1 * 7 + p2) * 72:(p1 * 7 + p2 + 1) * 72, :] = w
            return token(w)

        return [(40, lambda p1=p1, p2=p2: piece(p1, p2)) for p1 in ORDER for p2 in ORDER]

    def long_conv(i):
        kv, spec = {}, {}
        lane = lambda n: lax.broadcasted_iota(jnp.int32, (n, 128), 1)
        zrow = lambda r, sig, n, c, h: ((r % CB // 8) * 65 + sig * 32 + n * 8 + c * 2 + h) * 8

        def quarters(p):
            ln = lane(p[0].shape[0])
            even, low, mid = (ln & 32) == 0, ln < 64, ((ln + 32) & 64) != 0
            r0, r1 = jnp.where(even, p[0], p[1]), jnp.where(even, p[2], p[3])
            r2, r3 = jnp.where(even, p[1], p[0]), jnp.where(even, p[3], p[2])
            return [jnp.where(low, r0, r1), jnp.where(mid, r2, r3), jnp.where(low, r1, r0), jnp.where(mid, r3, r2)]

        def to_phases(v):
            ln = lane(v[0].shape[0])
            return quarters([jnp.take_along_axis(v[a], 4 * (ln & 31) + (((ln >> 5) - a) & 3), axis=1) for a in range(4)])

        def from_phases(x):
            ln = lane(x[0].shape[0])
            return [jnp.take_along_axis(p, 32 * ((ln + a) & 3) + (ln >> 2), axis=1) for a, p in enumerate(quarters(x))]

        def short_conv(r, a):
            cur = k_v[i, r // 2:r // 2 + 8, a * CH:(a + 1) * CH]
            old = k_v[i, r // 2:r // 2 + 8, (a - 1) * CH:a * CH] if a else jnp.zeros((8, CH), u32)
            taps = [_rows2(cur)] + [_rows2(jnp.where(lane(8) >= j, pltpu.roll(cur, j, 1), pltpu.roll(old, j, 1)))
                                    for j in range(1, 4)]
            vv = _rows2(v_v[i, r // 2:r // 2 + 8, a * CH:(a + 1) * CH])
            x = []
            for h in range(2):
                rows = pl.ds(pl.multiple_of(i * CS, CS) + r + h, 8, stride=2)
                ks = taps[0][h] * cols[0, rows, :]
                for j in range(1, 4):
                    ks = ks + taps[j][h] * cols[j, rows, :]
                x.append(ks * vv[h])
            kv[r, a] = _join2(*x)
            return kv[r, a]

        def spectra(r0, sig):
            rs = range(r0, r0 + CB, 16)
            if sig == 0:
                get = lambda r, a: ssmk_v[i, r // 2:r // 2 + 8, a * CH:(a + 1) * CH]
            else:
                get = lambda r, a: kv[r, a]
            ph = {(c, r): to_phases([get(r, 4 * c + a) for a in range(4)]) for c in range(4) for r in rs}
            zb = zbs[r0 // CB]
            for odd in range(2):
                z = [jnp.dot(_unpack(jnp.concatenate([ph[c, r][f] for c in range(4) for r in rs], axis=0)),
                             _unpack(fmat[f]), preferred_element_type=f32) for f in (odd, odd + 2)]
                for n, v in enumerate((z[0] + z[1], z[0] - z[1])):
                    for c in range(4):
                        for r in range(0, CB, 8):
                            for h in range(2):
                                row = zrow(r, sig, 2 * odd + n, c, h)
                                zb[row:row + 8, :] = v[c * CB + r:c * CB + r + 8, h * CH:(h + 1) * CH]

        def loader(r):
            zb, r16 = zbs[r // CB], r // 16 * 16

            def load(sig, n, c, h):
                return zb[pl.ds(zero(0) + zrow(r, sig, n, c, h), 8), :]
            return load

        ext = {}

        def spectrum(r, sig, l, c):
            if (r, sig, l, c) not in ext:
                load = loader(r)
                ar, ai = load(sig, l % 2, c, 0), load(sig, l % 2, c, 1)
                br, bi = load(sig, 2 + l % 2, c, 0), load(sig, 2 + l % 2, c, 1)
                ext[r, sig, l, c] = [(ar + br, ai + bi), (ar - bi, ai + br), (ar - br, ai - bi), (ar + bi, ai - br)][l]
            return ext[r, sig, l, c]

        def window(r, l, c):
            if (r, 2, l, c) not in ext:
                kr, ki = spectrum(r, 0, l, c)
                if c:
                    pr, pi = spectrum(r, 0, l, c - 1)
                    ext[r, 2, l, c] = (kr + pi, ki - pr)
                else:
                    ext[r, 2, l, c] = (kr + cols[4, pl.ds(pl.multiple_of(i * CS, CS) + r, 8), :], ki)
            return ext[r, 2, l, c]

        def product(r, l, c):
            yr = yi = None
            for j in range(c + 1):
                (kr, ki), (ur, ui) = window(r, l, j), spectrum(r, 1, l, c - j)
                tr, ti = kr * ur - ki * ui, kr * ui + ki * ur
                yr, yi = (tr, ti) if j == 0 else (yr + tr, yi + ti)
            ext[r, 3, l, c] = (yr, yi)
            if l < 2:
                return yr + yi
            (ar, ai), (br, bi) = ext[r, 3, l - 2, c], (yr, yi)
            ext[r, 4, l - 2, c] = (ar + br, ai + bi, ar - br, ai - bi)
            if l == 2:
                return ext[r, 4, 0, c][2] + ext[r, 4, 0, c][3]
            (s0r, s0i, d0r, d0i), (s1r, s1i, d1r, d1i) = ext[r, 4, 0, c], ext[r, 4, 1, c]
            for f, v in enumerate(((s0r + s1r, s0i + s1i), (d0r + d1i, d0i - d1r),
                                   (s0r - s1r, s0i - s1i), (d0r - d1i, d0i + d1r))):
                spec[f, c, r] = jnp.concatenate(v, axis=1)
            return spec[3, c, r][:, :CH] + spec[3, c, r][:, CH:]

        def inverse(r0):
            y = [jnp.dot(jnp.concatenate([spec[f, c, r] for c in range(4) for r in range(r0, r0 + CI, 8)],
                                         axis=0).astype(bf16),
                         _unpack(gmat[f]), preferred_element_type=f32) for f in range(4)]
            rows = pl.ds(pl.multiple_of(i * CS, CS) + r0, CI)
            for b in range(NT):
                yb = jnp.concatenate(from_phases([y[f][b * CI:(b + 1) * CI, :] for f in range(4)]), axis=1)
                g = g_v[0:1, b * T:(b + 1) * T]
                ga_v[b, rows, :] = g * (q_v[b, rows, :].astype(f32) * yb) + (1.0 - g) * x1_v[b, rows, :]

        return ([[(30, lambda r=r, a=a: short_conv(r, a)) for a in range(NCH)] for r in range(0, CS, 16)],
                [[(0, lambda r=r: spectra(r, 0))] for r in range(0, CS, CB)],
                [[(0, lambda r=r: spectra(r, 1))] for r in range(0, CS, CB)],
                [[(8 * c + 12, lambda r=r + h, l=l, c=c: product(r, l, c))
                  for h in (0, 8) for l in (0, 2, 1, 3) for c in range(4)] for r in range(0, CS, 16)],
                lambda: [inverse(r) for r in range(0, CS, CI)])

    def up(i, t, p1, due):
        if t == 0:
            w3_operands(i, p1)
        pv = {}
        for p2 in _UP_ORDER:
            p = p1 * 7 + p2
            n = TILE0[p + 1] - TILE0[p]
            a = jnp.concatenate([_unpack(tied(xa[zero(5) + t, TILE0[p] + j], next(due))) for j in range(n)], axis=1)
            bt = [_unpack(wb[zero(1 + t) + TILE0[p] + j, :min(64, DEPTH[p] * 32 - 64 * j), :]) for j in range(n)]
            pv[p2] = jnp.dot(a[:, :DEPTH[p] * 64], jnp.concatenate(bt, axis=0), preferred_element_type=f32)
        for q, c in enumerate(_combine7(pv)):
            pb[t][(p1 * 4 + q) * MP:(p1 * 4 + q) * MP + 128, :] = c

    def down(t, due):
        hid = {}

        def hidden(k, s):
            if (k, s) not in hid:
                q, q2 = (s // 2) * 2 + k // 2, (s % 2) * 2 + k % 2
                hid[k, s] = _gelu_u(_lin([(SC[p1, q], pb[t][pl.ds(zero(0) + (p1 * 4 + q2) * MP, 128), :])
                                          for p1 in range(7) if SC[p1, q]]))
            return hid[k, s]

        for p1 in ORDER:
            for p2 in ORDER:
                p = p1 * 7 + p2
                hv = _lin([(c * c2, hidden(2 * k + r, 2 * j + s))
                           for (k, j), c in SB[p1].items() for (r, s), c2 in SB[p2].items()])
                y = lax.dot_general(_unpack(tied(wa[pl.ds(zero(1 + t) + p * 72, 72), :], next(due))), hv.astype(bf16),
                                    (((1,), (1,)), ((), ())), preferred_element_type=f32)
                acc[t][p * MP:(p + 1) * MP, :] += y

    def finish(t):
        def piece(r):
            og = (1.0 - g_v[0:1, t * T:(t + 1) * T]) * KAPPA
            c = _combine(lambda p: acc[t][pl.ds(zero(0) + p * MP + r, 16), :], 2)
            tok = None
            for m in range(4):
                rows = slice(m * MP + r, m * MP + r + 16)
                out = ga_v[t, rows, :] + og * jnp.concatenate(c[m], axis=1)
                o_v[t, rows, :] = out.astype(bf16)
                tok = out[:8, m * 128:(m + 1) * 128] if tok is None else tok + out[8:, m * 128:(m + 1) * 128]
            if r + 16 == MP:
                cp_out[t].start()
            return tok
        return [(256, lambda r=r: piece(r)) for r in range(0, MP, 16)]

    idle = lambda n: [[]] * n

    def ups(i, t, due):
        due = iter(due)
        for p1 in range(7):
            up(i, t, p1, due)

    def chunk(i):
        kv, filt, data, mac, inverse = long_conv(i + 1)
        v = w4_operands(i)
        early = filt[0] + kv[0] + filt[1] + kv[1] + kv[2][:4] + data[0] + kv[2][4:] + kv[3] + v[:4] + data[1] + v[4:]
        prods = mac[0] + mac[1] + mac[2] + mac[3]
        nl, ml = 0, 40
        due = schedule(early + prods[:len(prods) - nl], 3 * NTILE)
        for t in range(1, NT):
            ups(i, t, due[(t - 1) * NTILE:t * NTILE])
        if not nl:
            inverse()
        for t in range(NT):
            down(t, iter(idle(NPROD)))
        ups(i + 1, 0, schedule(prods[len(prods) - nl:], ml) + idle(NTILE - ml) if nl else idle(NTILE))
        if nl:
            inverse()

    def last_chunk(i):
        fs = 8
        ups(i, 1, schedule(w4_operands(i), NTILE))
        down(0, iter(idle(NPROD)))
        ups(i, 2, idle(fs) + schedule(finish(0), NTILE - fs))
        down(1, iter(idle(NPROD)))
        ups(i, 3, idle(fs) + schedule(finish(1), NTILE - fs))
        down(2, iter(idle(NPROD)))
        down(3, iter(idle(fs) + schedule(finish(2), NPROD - fs)))
        for _, fn in finish(3):
            fn()

    if 0 == 1:
        def body0(i, c):
            chunk(i)
            return c
        lax.fori_loop(0, NF - 1, body0, 0)
        o_v[0, :16, :128] = sum(r[pl.ds(zero(0), 16), :] for r in zbs + pb + acc).astype(bf16) + ga_v[zero(0), :16, :128].astype(bf16) + _unpack(wa[pl.ds(zero(0), 8), :])
        cp_out[0].start(); cp_out[0].wait()
        return
    if 0 == 2:
        last_chunk(NF - 1)
        for cp in cp_out:
            cp.wait()
        return
    head = [cp_w1, cp_q[0], cp_q[1]]
    for cp in head:
        cp.start()

    sk = sk_ref[...].astype(f32)
    for j in range(4):
        cols[j] = _col(sk[j:j + 1, :])
    cols[4] = _col(ssmd_ref[...].astype(f32).reshape(1, D))
    cols[5] = _col(gw_ref[...].astype(f32).reshape(1, D))

    order = ([(1, n) for n in range(12)] + [(2, n) for n in range(4)] + [(1, n) for n in range(12, 16)]
             + [(2, n) for n in range(4, 16)])
    times = [n / TIES for n in range(len(order) * TIES)] + [len(order) + n * 32 / 720 for n in range(NTILE)]
    due = [[] for _ in times]

    def place(pieces, d0, d1):
        slots = [n for n, d in enumerate(times) if d0 <= d < d1]
        for slot, fns in zip(slots, schedule(pieces, len(slots))):
            due[slot] += fns

    def w2_part(j):
        n = min(128, D - 128 * j)
        w = w2_v[:, 128 * j:128 * j + n].astype(f32)
        w = jnp.concatenate([w, jnp.zeros((64, n), f32)], axis=0)
        if n < 128:
            w = jnp.concatenate([w, jnp.zeros((D + 64, 128 - n), f32)], axis=1)
        w = pltpu.bitcast(w.astype(bf16).T, u32)[:n // 2]
        w2t[0, 64 * j:64 * j + n // 2, :] = w
        return w[:8, 512:]

    b1, b2, ready = 7, 12, 0
    kv, filt, data, mac, inverse = long_conv(0)
    place([(18, lambda j=j: clear(j)) for j in range(NT * NPROD)], 0, 20)
    place([(1, lambda j=j: w2_part(j)) for j in range(5)], b1 + 1, 11)
    k1 = b2 + 4
    place(filt[0] + kv[0] + kv[1] + filt[1] + kv[2] + kv[3] + data[0] + data[1], b2 + 0.5, k1)
    place(mac[0] + mac[1] + mac[2] + mac[3], k1 + 1, 29)
    for d, (stage, n) in enumerate(order):
        if stage == 1 and d:
            place(stats1(n), d - 1, d - 3 / 10)

    for cp in head:
        cp.wait()
    second = [cp_q[2], cp_q[3], cp_w2]
    third = [pltpu.make_async_copy(f_hbm, fmat, sem_w.at[2]), pltpu.make_async_copy(g_hbm, gmat, sem_w.at[3]),
             cp_mlp(0)[0]] + cp_conv(0)
    for cp in second:
        cp.start()
    w1t[0] = transposed(w1_v[...])
    for _, fn in stats1(0):
        fn()
    for d, (stage, n) in enumerate(order):
        if d == b1:
            for cp in second:
                cp.wait()
            for cp in third:
                cp.start()
        if d == b2:
            for cp in third:
                cp.wait()
            for cp in [cp_mlp(0)[1]] + cp_conv(1) + cp_mlp(1) + cp_conv(2):
                cp.start()
        one, two = (stage1, stage2)[stage - 1](n, due[d * TIES:(d + 1) * TIES])
        lag, lag2 = 13 / 10, 12 / 10
        if d >= 30:
            lag, lag2 = 12 / 10, 6 / 10
        place(one, d + lag, d + lag + min(1, lag2))
        if two:
            place(two, d + lag + lag2, d + lag + lag2 + min(1, lag2))
            ready = max(ready, d + lag + lag2 + min(1, lag2))
        if stage == 2 and n % 4 == 3:
            place(x_operands(n // 4), ready, ready + 3)
    ups(0, 0, due[len(order) * TIES:])
    inverse()
    if 0 == 3:
        o_v[0, :16, :128] = _unpack(xa[zero(0), 0, :8, :]) + sum(r[pl.ds(zero(0), 16), :] for r in acc + pb).astype(bf16) + ga_v[zero(0), :16, :128].astype(bf16)
        cp_out[0].start(); cp_out[0].wait()
        return

    def body(i, c):
        for cp in [cp_mlp(i)[1], cp_mlp(i + 1)[0]] + cp_conv(i + 1):
            cp.wait()

        @pl.when(i + 2 < NF)
        def _():
            for cp in cp_mlp(i + 2):
                cp.start()

        @pl.when(i + 3 < NF)
        def _():
            for cp in cp_conv(i + 3):
                cp.start()

        chunk(i)
        return c

    lax.fori_loop(0, NF - 1, body, 0)
    cp_mlp(NF - 1)[1].wait()
    last_chunk(NF - 1)
    for cp in cp_out:
        cp.wait()


@jax.jit
def pallas_gated_mix__ssm_conv_h3__mixer_s_mlp__prompt_kernel(A_q, A_k, A_v, A_shift_k, A_ssm_k, A_ssm_D, B_x, B_w1, B_w2, B_w3, B_w4, gate_w):
    del B_x
    hbm = pl.BlockSpec(memory_space=pl.ANY)
    vmem = pl.BlockSpec(memory_space=pltpu.VMEM)
    out = pl.pallas_call(
        _kernel,
        out_shape=jax.ShapeDtypeStruct((D, S), bf16),
        in_specs=[pl.BlockSpec(memory_space=pltpu.SMEM), hbm, hbm, hbm, vmem, hbm, vmem, hbm, hbm, hbm, hbm, vmem, hbm, hbm],
        out_specs=hbm,
        scratch_shapes=[
            pltpu.VMEM((NT, D, T), bf16),
            *[pltpu.VMEM((NF, CS // 2, S), u32)] * 3,
            pltpu.VMEM((D, D), bf16), pltpu.VMEM((D, D), bf16),
            pltpu.VMEM((NF, D // 2, FC), u32), pltpu.VMEM((NF, D // 2, FC), u32),
            pltpu.VMEM((1, D // 2, 640), u32), pltpu.VMEM((1, D // 2, 640), u32),
            pltpu.VMEM((6, D, 128), f32),
            pltpu.VMEM((4, CH // 2, 2 * CH), u32), pltpu.VMEM((4, CH, CH), u32),
            pltpu.VMEM((D, S), f32), pltpu.VMEM((8, S), f32),
            pltpu.VMEM((NT, D, T), f32), pltpu.VMEM((NT, D, T), f32), pltpu.VMEM((NT, D, T), bf16),
            pltpu.VMEM((NT, NTILE, 64, 128), u32), pltpu.VMEM((NTILE, 64, 128), u32),
            pltpu.VMEM((NPROD * MP // 2, 128), u32), *[pltpu.VMEM((NPROD * MP, 128), f32)] * NT,
            *[pltpu.VMEM((65 * CB, CH), f32)] * 4,
            pltpu.VMEM((D, T), f32), pltpu.VMEM((D, T), f32),
        ] + [pltpu.VMEM((28 * MP, 128), f32)] * NT + [
            pltpu.SemaphoreType.DMA((NT,)), pltpu.SemaphoreType.DMA((4,)),
            pltpu.SemaphoreType.DMA((3, NF)), pltpu.SemaphoreType.DMA((2, NF)),
            pltpu.SemaphoreType.DMA((NT,)),
        ],
        compiler_params=pltpu.CompilerParams(vmem_limit_bytes=124 * 2**20),
    )(np.zeros((16,), np.int32), A_q[0].T, A_k[0].T, A_v[0].T, A_shift_k.T, A_ssm_k, A_ssm_D,
      B_w1, B_w2, B_w3, B_w4.T, gate_w, *_transform_tables())
    return out.T[None]
```

```python
import math
import numpy as np
import jax
import jax.numpy as jnp
from jax import lax
import jax.experimental.pallas as pl
import jax.experimental.pallas.tpu as pltpu

S, D, F = 2048, 576, 4608
CH = 128
NCH = S // CH
f32, bf16, u32 = jnp.float32, jnp.bfloat16, jnp.uint32

T = 512
NT = S // T
FC = 512
NF = F // FC
CS = D // NF
TIES = 12
MP = D // 4
PS, AS, XS = 136, 2 * MP + 8, 72
QT, FR = 6, 32
CB, CI = 32, 64
ORDER = (1, 4, 0, 2, 5, 3, 6)

_C0 = math.sqrt(2.0 / math.pi)
GS = (_C0 * 0.044715) ** (1.0 / 3.0)
GK = _C0 / GS
KAPPA = 0.5 / GS

SA = [{(0, 0): 1, (1, 1): 1}, {(1, 0): 1, (1, 1): 1}, {(0, 0): 1}, {(1, 1): 1},
      {(0, 0): 1, (0, 1): 1}, {(1, 0): 1, (0, 0): -1}, {(0, 1): 1, (1, 1): -1}]
SB = [{(0, 0): 1, (1, 1): 1}, {(0, 0): 1}, {(0, 1): 1, (1, 1): -1}, {(1, 0): 1, (0, 0): -1},
      {(1, 1): 1}, {(0, 0): 1, (0, 1): 1}, {(1, 0): 1, (1, 1): 1}]
SC = np.array([[1, 0, 0, 1], [0, 0, 1, -1], [0, 1, 0, 1], [1, 0, 1, 0], [-1, 1, 0, 0], [0, 0, 0, 1], [1, 0, 0, 0]])


def _single(ps):
    inv = np.rint(np.linalg.inv(SC[list(ps)].astype(np.float64))).astype(int)
    out = {}
    for n, p in enumerate(ps):
        lam = inv[:, n].reshape(2, 2)
        i0, j0 = np.argwhere(lam != 0)[0]
        a, b = lam[:, j0] * lam[i0, j0], lam[i0, :].copy()
        assert (np.outer(a, b) == lam).all()
        if (b <= 0).all():
            a, b = -a, -b
        out[p] = ({i: int(a[i]) for i in range(2) if a[i]}, {j: int(b[j]) for j in range(2) if b[j]})
    return out


_PLAN = {9: (3, [(1, 3, 2, 5), (2, 4, 3, 6), (0, 3, 2, 5)]), 4: (2, []),
         6: (2, [(0, 1, 2, 5), (0, 1, 2, 5)]), 5: (1, [(1, 3, 2, 5), (2, 4, 1, 5), (0, 1, 2, 5)])}


def _level(depth):
    n_pairs, singles = _PLAN[depth]
    terms = [[] for _ in range(7)]
    for t in range(n_pairs):
        kk = (2 * t, 2 * t + 1)
        for p in range(7):
            terms[p].append(({(i, kk[k]): c for (i, k), c in SA[p].items()},
                             {(j, kk[k]): c for (k, j), c in SB[p].items()}))
    for n, ps in enumerate(singles):
        kb = 2 * n_pairs + n
        for p, (a, b) in _single(ps).items():
            terms[p].append(({(i, kb): c for i, c in a.items()}, {(j, kb): c for j, c in b.items()}))
    return terms


def _lin(items):
    acc = None
    for c, v in sorted(items, key=lambda cv: -cv[0]):
        if acc is None:
            acc = v if c > 0 else -v
        else:
            acc = acc + v if c > 0 else acc - v
    return acc


def _deep_operands(blocks, side, levels):
    if levels == 0:
        return [[b[0] for b in blocks]]
    h = len(blocks[0]) // 2
    out = []
    for terms in _level(len(blocks)):
        nxt = [[_lin([(c, blocks[kb][i * h + s]) for (i, kb), c in t[side].items()]) for s in range(h)]
               for t in terms]
        out += _deep_operands(nxt, side, levels - 1)
    return out


def _deep_group(get, side, p1):
    terms = _level(9)[p1]
    nxt = [[_lin([(c, get(kb, i * 2 + s)) for (i, kb), c in t[side].items()]) for s in range(2)] for t in terms]
    return _deep_operands(nxt, side, 1)


class _Sum(dict):
    def __add__(self, other):
        return _Sum({k: v for k in {**self, **other} if (v := self.get(k, 0) + other.get(k, 0))})

    def __neg__(self):
        return _Sum({k: -v for k, v in self.items()})

    def __sub__(self, other):
        return self + -other


_X_TERMS = _deep_operands([[_Sum({(kb, s): 1}) for s in range(4)] for kb in range(9)], 0, 2)
_UP_ORDER = (1, 3, 2, 4, 0, 5, 6)


def _combine7(p):
    return [(p[3] - p[4]) + p[0] + p[6], p[2] + p[4], p[1] + p[3], (p[2] - p[1]) + p[0] + p[5]]


DEPTH = [len(t2) for t1 in _level(9) for t2 in _level(len(t1))]
NPROD = len(DEPTH)
TILE0 = [sum((d + 1) // 2 for d in DEPTH[:p]) for p in range(NPROD + 1)]
NTILE = TILE0[-1]


def _unpack(v):
    return pltpu.bitcast(v, bf16)


def _rows2(w):
    return [pltpu.unpack_elementwise(w, index=i, packed_dtype=bf16, unpacked_dtype=f32) for i in range(2)]


def _join2(even, odd):
    return pltpu.pack_elementwise([even, odd], packed_dtype=bf16)


def _gelu_u(u):
    return u + u * jnp.tanh(u * (u * u + GK))


def _col(row):
    b = jnp.broadcast_to(row, (128, D))
    b = jnp.concatenate([b, jnp.zeros((128, 64), f32)], axis=1)
    return b.T[:D, :]


def _transform_tables():
    def words(x):
        bits = x.astype(bf16).view(np.uint16).astype(np.uint32)
        return bits[:, 0::2] | (bits[:, 1::2] << 16)
    f, lane, m = np.ogrid[:4, :CH, :CH]
    angle = ((4 * m + 1) * (4 * ((lane - 32 * f) % CH) + f) % 2048) * (np.pi / 1024.0)
    fwd = np.concatenate([np.cos(angle), np.sin(angle)], axis=2)
    return words(fwd), words(fwd.transpose(0, 2, 1) / T)


def _kernel(q_hbm, k_hbm, v_hbm, sk_hbm, ssmk_hbm, ssmd_hbm, w1_hbm, w2_hbm, w3_hbm, w4_hbm, gw_hbm,
            zero_hbm, f_hbm, g_hbm, out_hbm,
            zero_ref,
            q_v, k_v, v_v, ssmk_v, w3_v, w4_v, w1t, w2t, cols, fmat, gmat,
            h_v, g_v, x1_v, ga_v, o_v, xa, wb, wa, zb0, zb1, xn0, xn1, pb0, pb1, pb2, pb3,
            sem_q, sem_w, sem_c, sem_f, sem_out, *rest):
    *acc, w1_v, w2_v, sk_ref, ssmd_ref, gw_ref = rest
    pb = (pb0, pb1, pb2, pb3)
    xnb = (xn0, xn1)
    zbs = (zb0, zb1)
    cp_q = [pltpu.make_async_copy(q_hbm.at[:, pl.ds(b * T, T)], q_v.at[b], sem_q.at[b]) for b in range(NT)]
    cp_w1 = pltpu.make_async_copy(w1_hbm, w1_v, sem_w.at[0])
    cp_w2 = pltpu.make_async_copy(w2_hbm, w2_v, sem_w.at[1])
    cp_out = [pltpu.make_async_copy(
        o_v.at[n], out_hbm.at[pl.ds(n % 4 // 2 * 2 * MP, 2 * MP), pl.ds(n // 4 * T + n % 2 * 256, 256)], sem_out.at[n])
        for n in range(4 * NT)]

    def weights(n, chunks, sem):
        src, dst = ((w3_hbm, w3_v), (w4_hbm, w4_v))[n]
        return [pltpu.make_async_copy(src.bitcast(u32).at[:, pl.ds(i * FC, FC)], dst.at[i], sem) for i in chunks]

    def conv_inputs(first, count, group):
        words = pl.ds(first * (CS // 2), count * (CS // 2))
        return [pltpu.make_async_copy(src.bitcast(u32).at[words, :], dst.at[words, :], sem_c.at[group, n])
                for n, (src, dst) in enumerate(((k_hbm, k_v), (v_hbm, v_v), (ssmk_hbm, ssmk_v)))]

    aligned = lambda x, n: x if isinstance(x, int) else pl.multiple_of(x, n)

    def zero(n):
        return pl.multiple_of(zero_ref[n], 64)

    def schedule(pieces, slots):
        total, now, out = sum(w for w, _ in pieces), 0, [[] for _ in range(slots)]
        for w, fn in pieces:
            out[min(slots - 1, int((now + w / 2) * slots / total))].append(fn)
            now += w
        return out

    def both(*plans):
        return [[fn for part in slot for fn in part] for slot in zip(*plans, strict=True)]

    def tied(w, *due):
        step = w.shape[0] // 8 // len(due) * 8
        parts = []
        for j, fns in enumerate(due):
            tie = None
            for fn in fns:
                t = fn()
                if t is not None:
                    t = pltpu.bitcast(t, u32)
                    tie = t if tie is None else tie | t
            top = w[j * step:j * step + 8]
            if tie is not None:
                left = top[:, :128] | (tie & jnp.full((8, 128), zero_ref[0], jnp.int32).astype(u32))
                top = jnp.concatenate([left, top[:, 128:]], axis=1) if w.shape[1] > 128 else left
            parts += [top, w[j * step + 8:(j + 1) * step if j + 1 < len(due) else w.shape[0]]]
        return jnp.concatenate(parts, axis=0)

    def token(w):
        t = w[:8, :128]
        for r in range(8, w.shape[0], 8):
            t = t | w[r:r + 8, :128]
        return t

    def transposed(w):
        w = w.astype(f32)
        w = jnp.concatenate([w, jnp.zeros((D, 64), f32)], axis=1)
        w = jnp.concatenate([w, jnp.zeros((64, D + 64), f32)], axis=0)
        return pltpu.bitcast(w.astype(bf16).T, u32)[:D // 2, :]

    def moments(state, x):
        if not state:
            state.update(pivot=jnp.broadcast_to(x[:1], (8, 128)), s1=None, s2=None)
        for r in range(0, x.shape[0], 8):
            d = x[r:r + 8] - state['pivot']
            state['s1'] = d if state['s1'] is None else state['s1'] + d
            state['s2'] = d * d if state['s2'] is None else state['s2'] + d * d

    def mean_scale(state):
        m = jnp.sum(state['s1'], axis=0, keepdims=True) * (1.0 / D)
        v = jnp.sum(state['s2'], axis=0, keepdims=True) * (1.0 / D) - m * m
        state['mean'] = state['pivot'] + m
        state['scale'] = jnp.broadcast_to(lax.rsqrt(jnp.maximum(v, 0.0) + 1e-5) * GS, (8, 128))
        return state['scale']

    def normalized(state, x):
        return jnp.concatenate([(x[r:r + 8] - state['mean']) * state['scale'] for r in range(0, x.shape[0], 8)], axis=0)

    stats = [{} for _ in range(S // 128)]

    def stats1(n):
        b, s = divmod(n, 4)
        gate = []

        def piece(r):
            x = q_v[b + zero(0), r:r + 48, s * 128:(s + 1) * 128].astype(f32)
            moments(stats[n], x)
            xw = x * cols[5, r:r + 48, :]
            for j in range(0, 48, 8):
                gate[:] = [xw[j:j + 8] + gate[0] if gate else xw[j:j + 8]]
            if r + 48 < D:
                return stats[n]['s2'] + gate[0]
            g = jnp.broadcast_to(jax.nn.sigmoid(jnp.sum(gate[0], axis=0, keepdims=True)), (8, 128))
            g_v[:, n * 128:(n + 1) * 128] = g
            return mean_scale(stats[n]) + g
        return [(42, lambda r=r: piece(r)) for r in range(0, D, 48)]

    def stage1(n, due, sync):
        b, s = divmod(n, 4)
        x = normalized(stats[n], q_v[b + zero(1), :, s * 128:(s + 1) * 128].astype(f32)).astype(bf16)
        sync()
        z = jnp.dot(_unpack(tied(w1t[zero(0), :D // 2, :], *due))[:, :D], x, preferred_element_type=f32)

        def act(r):
            h = _gelu_u(z[r:r + 48])
            h_v[r:r + 48, n * 128:(n + 1) * 128] = h
            return h_v[pl.ds(zero(0), 8), :128]
        return [(36, lambda r=r: act(r)) for r in range(0, D, 48)], []

    def stage2(n, due, sync):
        grp = D // 4
        b, s = divmod(n, 4)
        c0 = n * 128
        w = _unpack(tied(w2t[zero(0), :D // 2, :], *due))[:, :D]
        parts = []
        for gi, k in enumerate((1, -1, 2, -2)):
            rows = slice(gi * grp, (gi + 1) * grp)
            cur = h_v[rows, c0:c0 + 128]
            if k > 0:
                halo = h_v[rows, c0 - 128:c0] if c0 > 0 else jnp.zeros((grp, 128), f32)
                parts.append(pltpu.roll(jnp.concatenate([halo, cur], axis=1), k, 1)[:, 128:])
            else:
                halo = h_v[rows, c0 + 128:c0 + 256] if c0 + 128 < S else jnp.zeros((grp, 128), f32)
                parts.append(pltpu.roll(jnp.concatenate([cur, halo], axis=1), 256 + k, 1)[:, :128])
        z = jnp.dot(w, jnp.concatenate(parts, axis=0).astype(bf16), preferred_element_type=f32)
        c = slice(s * 128, (s + 1) * 128)
        state = {}

        def residual(r):
            x1 = q_v[b + zero(2), r:r + 48, c].astype(f32) + z[r:r + 48]
            x1_v[b, r:r + 48, c] = x1
            moments(state, x1)
            return state['s2'] if r + 48 < D else mean_scale(state)

        def norm(r):
            row = (s * 9 + r // 64) * XS
            xnb[b % 2][row:row + 64, :] = normalized(state, x1_v[b + zero(0), r:r + 64, c])
            return xnb[b % 2][pl.ds(zero(0), 8), :]
        return ([(40, lambda r=r: residual(r)) for r in range(0, D, 48)],
                [(24, lambda r=r: norm(r)) for r in range(0, D, 64)])

    def x_operands(b):
        def piece(p, n):
            pair = [_lin([(c, xnb[b % 2][pl.ds(zero(8 + p % 7) + (s * 9 + kb) * XS, 64), :])
                          for (kb, s), c in terms.items()]) for terms in _X_TERMS[p][2 * n:2 * n + 2]]
            if len(pair) == 1:
                pair.append(jnp.zeros((64, 128), f32))
            w = pltpu.bitcast(jnp.concatenate(pair, axis=0).astype(bf16).T, u32)
            xa[b, TILE0[p] + n] = w
            return w[56:]

        return [(4 + sum(map(len, _X_TERMS[p][2 * n:2 * n + 2])), lambda p=p, n=n: piece(p, n))
                for p in range(NPROD) for n in range(TILE0[p + 1] - TILE0[p])]

    def w3_operands(i):
        groups = {}

        def piece(p, n):
            p1, p2 = divmod(p, 7)
            if p1 not in groups:
                ii = i + zero(8 + p1)
                words = lambda kb, s: _rows2(w3_v[ii, kb * 32:(kb + 1) * 32, s * 128:(s + 1) * 128])
                groups[p1] = [_deep_group(lambda kb, s: words(kb, s)[h], 1, p1) for h in range(2)]
            w = _join2(groups[p1][0][p2][n], groups[p1][1][p2][n])
            wb[TILE0[p] + n // 2, (n % 2) * 32:(n % 2) * 32 + 32, :] = w
            return token(w)

        return [(17, lambda p=p, n=n: piece(p, n)) for p in range(NPROD) for n in range(DEPTH[p])]

    def w4_operands(i):
        def piece(p, r):
            words = [(c, _rows2(w4_v[i + zero(8 + p), m * MP + r:m * MP + r + 48, k * 256:(k + 1) * 256]))
                     for (m, k), c in SA[p].items()]
            w = _join2(*[_lin([(c, w[h]) for c, w in words]) for h in range(2)])
            wa[p * MP + r:p * MP + r + 48, :] = w
            return token(w[:, :128] | w[:, 128:])
        return [(40, lambda p=p, r=r: piece(p, r)) for p in ORDER if len(SA[p]) > 1 for r in range(0, MP, 48)]

    def long_conv(i):
        kv, spec = {}, {}
        words = lambda r: pl.ds(aligned(i * (CS // 2), CS // 2) + r // 2, 8)
        lane = lambda n: lax.broadcasted_iota(jnp.int32, (n, 128), 1)
        zrow = lambda r, sig, n, c, h: ((r % CB // 8) * 65 + sig * 32 + n * 8 + c * 2 + h) * 8

        def quarters(p):
            ln = lane(p[0].shape[0])
            even, low, mid = (ln & 32) == 0, ln < 64, ((ln + 32) & 64) != 0
            r0, r1 = jnp.where(even, p[0], p[1]), jnp.where(even, p[2], p[3])
            r2, r3 = jnp.where(even, p[1], p[0]), jnp.where(even, p[3], p[2])
            return [jnp.where(low, r0, r1), jnp.where(mid, r2, r3), jnp.where(low, r1, r0), jnp.where(mid, r3, r2)]

        def to_phases(v):
            ln = lane(v[0].shape[0])
            return quarters([jnp.take_along_axis(v[a], 4 * (ln & 31) + (((ln >> 5) - a) & 3), axis=1) for a in range(4)])

        def from_phases(x):
            ln = lane(x[0].shape[0])
            return [jnp.take_along_axis(p, 32 * ((ln + a) & 3) + (ln >> 2), axis=1) for a, p in enumerate(quarters(x))]

        def short_conv(r, a):
            cur = k_v[words(r), a * CH:(a + 1) * CH]
            old = k_v[words(r), (a - 1) * CH:a * CH] if a else jnp.zeros((8, CH), u32)
            taps = [_rows2(cur)] + [_rows2(jnp.where(lane(8) >= j, pltpu.roll(cur, j, 1), pltpu.roll(old, j, 1)))
                                    for j in range(1, 4)]
            vv = _rows2(v_v[words(r), a * CH:(a + 1) * CH])
            x = []
            for h in range(2):
                rows = pl.ds(aligned(i * CS, CS) + r + h, 8, stride=2)
                ks = taps[0][h] * cols[0, rows, :]
                for j in range(1, 4):
                    ks = ks + taps[j][h] * cols[j, rows, :]
                x.append(ks * vv[h])
            kv[r, a] = _join2(*x)
            return kv[r, a]

        def spectra(r0, sig):
            rs = range(r0, r0 + CB, 16)
            if sig == 0:
                get = lambda r, a: ssmk_v[words(r), a * CH:(a + 1) * CH]
            else:
                get = lambda r, a: kv[r, a]
            ph = {(c, r): to_phases([get(r, 4 * c + a) for a in range(4)]) for c in range(4) for r in rs}
            zb = zbs[r0 // CB]
            for odd in range(2):
                z = [jnp.dot(_unpack(jnp.concatenate([ph[c, r][f] for c in range(4) for r in rs], axis=0)),
                             _unpack(fmat[f]), preferred_element_type=f32) for f in (odd, odd + 2)]
                for n, v in enumerate((z[0] + z[1], z[0] - z[1])):
                    for c in range(4):
                        for r in range(0, CB, 8):
                            for h in range(2):
                                row = zrow(r, sig, 2 * odd + n, c, h)
                                zb[row:row + 8, :] = v[c * CB + r:c * CB + r + 8, h * CH:(h + 1) * CH]

        def loader(r):
            zb, r16 = zbs[r // CB], r // 16 * 16

            def load(sig, n, c, h):
                return zb[pl.ds(zero(0) + zrow(r, sig, n, c, h), 8), :]
            return load

        ext = {}

        def spectrum(r, sig, l, c):
            if (r, sig, l, c) not in ext:
                load = loader(r)
                ar, ai = load(sig, l % 2, c, 0), load(sig, l % 2, c, 1)
                br, bi = load(sig, 2 + l % 2, c, 0), load(sig, 2 + l % 2, c, 1)
                ext[r, sig, l, c] = [(ar + br, ai + bi), (ar - bi, ai + br), (ar - br, ai - bi), (ar + bi, ai - br)][l]
            return ext[r, sig, l, c]

        def window(r, l, c):
            if (r, 2, l, c) not in ext:
                kr, ki = spectrum(r, 0, l, c)
                if c:
                    pr, pi = spectrum(r, 0, l, c - 1)
                    ext[r, 2, l, c] = (kr + pi, ki - pr)
                else:
                    ext[r, 2, l, c] = (kr + cols[4, pl.ds(aligned(i * CS, CS) + r, 8), :], ki)
            return ext[r, 2, l, c]

        def product(r, l, c):
            yr = yi = None
            for j in range(c + 1):
                (kr, ki), (ur, ui) = window(r, l, j), spectrum(r, 1, l, c - j)
                tr, ti = kr * ur - ki * ui, kr * ui + ki * ur
                yr, yi = (tr, ti) if j == 0 else (yr + tr, yi + ti)
            ext[r, 3, l, c] = (yr, yi)
            if l < 2:
                return yr + yi
            (ar, ai), (br, bi) = ext[r, 3, l - 2, c], (yr, yi)
            ext[r, 4, l - 2, c] = (ar + br, ai + bi, ar - br, ai - bi)
            if l == 2:
                return ext[r, 4, 0, c][2] + ext[r, 4, 0, c][3]
            (s0r, s0i, d0r, d0i), (s1r, s1i, d1r, d1i) = ext[r, 4, 0, c], ext[r, 4, 1, c]
            for f, v in enumerate(((s0r + s1r, s0i + s1i), (d0r + d1i, d0i - d1r),
                                   (s0r - s1r, s0i - s1i), (d0r - d1i, d0i + d1r))):
                spec[f, c, r] = jnp.concatenate(v, axis=1)
            return spec[3, c, r][:, :CH] + spec[3, c, r][:, CH:]

        def inverse(r0):
            y = [jnp.dot(jnp.concatenate([spec[f, c, r] for c in range(4) for r in range(r0, r0 + CI, 8)],
                                         axis=0).astype(bf16),
                         _unpack(gmat[f]), preferred_element_type=f32) for f in range(4)]
            rows = pl.ds(aligned(i * CS, CS) + r0, CI)
            for b in range(NT):
                yb = jnp.concatenate(from_phases([y[f][b * CI:(b + 1) * CI, :] for f in range(4)]), axis=1)
                g = g_v[0:1, b * T:(b + 1) * T]
                ga_v[b, rows, :] = g * (q_v[b, rows, :].astype(f32) * yb) + (1.0 - g) * x1_v[b, rows, :]

        def inverse_all():
            for r in range(0, CS, CI):
                inverse(r)

        return ([[(30, lambda r=r, a=a: short_conv(r, a)) for a in range(NCH)] for r in range(0, CS, 16)],
                [[(0, lambda r=r: spectra(r, 0))] for r in range(0, CS, CB)],
                [[(0, lambda r=r: spectra(r, 1))] for r in range(0, CS, CB)],
                [[(8 * c + 12, lambda r=r + h, l=l, c=c: product(r, l, c))
                  for h in (0, 8) for l in (0, 2, 1, 3) for c in range(4)] for r in range(0, CS, 16)],
                inverse_all)

    def up(i, t, p1, due):
        pv = {}
        for p2 in _UP_ORDER:
            p = p1 * 7 + p2
            n = TILE0[p + 1] - TILE0[p]
            a = jnp.concatenate([_unpack(tied(xa[zero(5) + t, TILE0[p] + j], next(due))) for j in range(n)], axis=1)
            bt = [_unpack(wb[zero(1 + t) + TILE0[p] + j, :min(64, DEPTH[p] * 32 - 64 * j), :]) for j in range(n)]
            pv[p2] = jnp.dot(a[:, :DEPTH[p] * 64], jnp.concatenate(bt, axis=0), preferred_element_type=f32)
        for q, c in enumerate(_combine7(pv)):
            pb[t][(q * 7 + p1) * PS:(q * 7 + p1) * PS + 128, :] = c

    def down(i, t, due):
        hid = {}

        def hidden(k, s):
            if (k, s) not in hid:
                q, q2 = (s // 2) * 2 + k // 2, (s % 2) * 2 + k % 2
                hid[k, s] = _gelu_u(_lin([(SC[p1, q], pb[t][pl.ds(zero(0) + (q2 * 7 + p1) * PS, 128), :])
                                          for p1 in range(7) if SC[p1, q]]))
            return hid[k, s]

        for p in ORDER:
            if len(SA[p]) > 1:
                w = wa[pl.ds(zero(1 + t) + p * MP, MP), :]
            else:
                (m, k), = SA[p]
                w = w4_v[i + zero(1 + t), m * MP:(m + 1) * MP, k * 256:(k + 1) * 256]
            hv = jnp.concatenate([jnp.concatenate(
                [_lin([(c, hidden(2 * k + h, 2 * j + s)) for (k, j), c in SB[p].items()]) for h in range(2)], axis=1)
                for s in range(2)], axis=0)
            y = lax.dot_general(_unpack(tied(w, *[next(due) for _ in range(QT)])), hv.astype(bf16),
                                (((1,), (1,)), ((), ())), preferred_element_type=f32)
            for s in range(2):
                acc[2 * t + s][p * AS:p * AS + 2 * MP, :] += y[:, s * 128:(s + 1) * 128]

    def finish(t, q):
        def piece(r):
            rows = slice(q // 2 * 2 * MP + r, q // 2 * 2 * MP + r + FR)
            c0 = q % 2 * 256
            h2 = jnp.concatenate([_lin([(SC[p, q], acc[2 * t + s][pl.ds(zero(0) + p * AS + r, FR), :])
                                        for p in range(7) if SC[p, q]]) for s in range(2)], axis=1)
            og = (1.0 - g_v[0:1, t * T + c0:t * T + c0 + 256]) * KAPPA
            out = ga_v[t, rows, c0:c0 + 256] + og * h2
            o_v[4 * t + q, r:r + FR, :] = out.astype(bf16)
            return out[FR - 8:, :128] + out[FR - 16:FR - 8, 128:]
        return [(1, lambda r=r: piece(r)) for r in range(0, 2 * MP, FR)]

    def send(*blocks):
        def start():
            for n in blocks:
                cp_out[n].start()
        return [(0, start)]

    idle = lambda n: [[]] * n

    def ups(i, t, due):
        due = iter(due)
        for p1 in range(7):
            up(i, t, p1, due)

    def transforms(i):
        kv, filt, data, _, _ = long_conv(i)
        return filt[0] + kv[0] + filt[1] + kv[1] + kv[2][:4] + data[0] + kv[2][4:] + kv[3], data[1]

    def chunk(i, last=False):
        _, _, _, mac, inverse = long_conv(i)
        v = w4_operands(i)
        nm, sk = 16, 0
        mac = mac[0] + mac[1] + mac[2] + mac[3]
        due = idle(sk) + schedule(mac[:nm] + v + mac[nm:], 3 * NTILE - sk)
        for t in range(1, NT):
            ups(i, t, due[(t - 1) * NTILE:t * NTILE])
        if last:
            inverse()
            fs, lag = 8, 4
            whole = lambda t: finish(t, 1) + finish(t, 3) + finish(t, 2) + finish(t, 0)
            down(i, 0, iter(idle(7 * QT)))
            down(i, 1, iter(idle(fs) + schedule(whole(0) + send(0, 1, 2, 3), 7 * QT - fs)))
            down(i, 2, iter(idle(fs) + schedule(whole(1) + send(4, 5, 6, 7), 7 * QT - fs)))
            down(i, 3, iter(idle(fs) + schedule(whole(2) + send(8, 9, 10, 11), 4 * QT + lag - fs)
                            + schedule(finish(3, 1), QT) + schedule(finish(3, 3) + send(13, 15), QT)
                            + schedule(finish(3, 2), QT - lag)))
            for _, fn in send(14) + finish(3, 0) + send(12):
                fn()
            return
        q0, q1 = 6, 150
        due = iter(idle(q0) + schedule(w3_operands(i + 1), q1 - q0) + idle(28 * QT - q1))
        for t in range(NT):
            if t == 1:
                inverse()
            down(i, t, due)
        early, late = transforms(i + 1)
        te = 50
        ups(i + 1, 0, schedule(early, te) + idle(4) + [[late[0][1]]] + idle(NTILE))

    head = [cp_w1, cp_q[0]]
    small = [pltpu.make_async_copy(src, dst, sem_w.at[4 + n]) for n, (src, dst) in enumerate(
        ((zero_hbm, zero_ref), (sk_hbm, sk_ref), (ssmd_hbm, ssmd_ref), (gw_hbm, gw_ref)))]
    for cp in small + head:
        cp.start()
    for ref in acc[:4]:
        for p in range(7):
            ref[p * AS:p * AS + 2 * MP, :] = jnp.zeros((2 * MP, 128), f32)
    for cp in small:
        cp.wait()

    sk = sk_ref[...].astype(f32)
    for j in range(4):
        cols[j] = _col(sk[j:j + 1, :])
    cols[4] = _col(ssmd_ref[...].astype(f32).reshape(1, D))
    cols[5] = _col(gw_ref[...].astype(f32).reshape(1, D))
    for ref in acc[4:]:
        for p in range(7):
            ref[p * AS:p * AS + 2 * MP, :] = jnp.zeros((2 * MP, 128), f32)

    n1 = 13
    order = ([(1, n) for n in range(n1)] + [(2, n) for n in range(4)] + [(1, n) for n in range(n1, 16)]
             + [(2, n) for n in range(4, 16)])
    times = [n / TIES for n in range(len(order) * TIES)] + [len(order) + n * 32 / 720 for n in range(NTILE)]
    due = [[] for _ in times]

    def place(pieces, d0, d1):
        slots = [n for n, d in enumerate(times) if d0 <= d < d1]
        for slot, fns in zip(slots, schedule(pieces, len(slots))):
            due[slot] += fns

    def w2_part(j):
        n = min(128, D - 128 * j)
        w = w2_v[:, 128 * j:128 * j + n].astype(f32) * KAPPA
        w = jnp.concatenate([w, jnp.zeros((64, n), f32)], axis=0)
        if n < 128:
            w = jnp.concatenate([w, jnp.zeros((D + 64, 128 - n), f32)], axis=1)
        w = pltpu.bitcast(w.astype(bf16).T, u32)[:n // 2]
        w2t[0, 64 * j:64 * j + n // 2, :] = w
        return w[:8, 512:]

    ready = 0
    place([(1, lambda j=j: w2_part(j)) for j in range(5)], 11 + 2 / 10, n1 - 0.5)
    place(w3_operands(0), 13, 19)
    early, late = transforms(0)
    place([e for e in early if e[0]], 22, 27)
    place([(1, e[1]) for e in early if not e[0]], len(order), 99)
    for d, (stage, n) in enumerate(order):
        if stage == 1 and d:
            place(stats1(n), d - 1, d - 5 / 10)

    for cp in head:
        cp.wait()
    second = [cp_q[1], cp_q[2]]
    third = ([cp_q[3], cp_w2, pltpu.make_async_copy(f_hbm, fmat, sem_w.at[2])]
             + weights(0, [0], sem_f.at[0, 0]) + conv_inputs(0, 1, 0))
    fourth = ([pltpu.make_async_copy(g_hbm, gmat, sem_w.at[3])] + weights(0, [1, 2], sem_f.at[0, 1])
              + weights(1, [0, 1], sem_f.at[1, 1]) + conv_inputs(1, 2, 1))
    fifth = weights(0, range(3, NF), sem_f.at[0, 2]) + weights(1, range(2, NF), sem_f.at[1, 2]) + conv_inputs(3, NF - 3, 2)
    for cp in second:
        cp.start()
    w1t[0, :D // 2, :] = transposed(w1_v[...])
    for _, fn in stats1(0):
        fn()

    def sync(d):
        for cp in {3: second, 11: third}.get(d, []):
            cp.wait()
        if d == 3:
            for cp in third:
                cp.start()
        if d == 11:
            @pl.loop(0, 1 + zero_ref[0])
            def _(_):
                for cp in fourth:
                    cp.start()

    for d, (stage, n) in enumerate(order):
        one, two = (stage1, stage2)[stage - 1](n, due[d * TIES:(d + 1) * TIES], lambda: sync(d))
        lag, lag2 = 13 / 10, 12 / 10
        if d >= 31:
            lag, lag2 = 12 / 10, 6 / 10
        place(one, d + lag, d + lag + min(1, lag2))
        if two:
            place(two, d + lag + lag2, d + lag + lag2 + min(1, lag2))
            ready = max(ready, d + lag + lag2 + min(1, lag2))
        if stage == 2 and n % 4 == 3:
            place(x_operands(n // 4), ready, ready + 3)
    ups(0, 0, due[len(order) * TIES:])
    late[0][1]()
    for cp in fourth:
        cp.wait()
    for cp in fifth:
        cp.start()

    def arrived():
        for cp in fifth:
            cp.wait()

    @pl.loop(0, NF - 1)
    def _(i):
        pl.when(i == 2)(arrived)
        chunk(i)

    chunk(NF - 1, last=True)
    for cp in cp_out:
        cp.wait()


@jax.jit
def pallas_gated_mix__ssm_conv_h3__mixer_s_mlp__prompt_kernel(A_q, A_k, A_v, A_shift_k, A_ssm_k, A_ssm_D, B_x, B_w1, B_w2, B_w3, B_w4, gate_w):
    del B_x
    hbm = pl.BlockSpec(memory_space=pl.ANY)
    out = pl.pallas_call(
        _kernel,
        out_shape=jax.ShapeDtypeStruct((D, S), bf16),
        in_specs=[hbm] * 14,
        out_specs=hbm,
        scratch_shapes=[
            pltpu.SMEM((16,), jnp.int32),
            pltpu.VMEM((NT, D, T), bf16),
            *[pltpu.VMEM((D // 2, S), u32)] * 3,
            pltpu.VMEM((NF, D // 2, FC), u32), pltpu.VMEM((NF, D // 2, FC), u32),
            pltpu.VMEM((1, 320, 640), u32), pltpu.VMEM((1, 320, 640), u32),
            pltpu.VMEM((6, D, 128), f32),
            pltpu.VMEM((4, CH // 2, 2 * CH), u32), pltpu.VMEM((4, CH, CH), u32),
            pltpu.VMEM((D, S), f32), pltpu.VMEM((8, S), f32),
            pltpu.VMEM((NT, D, T), f32), pltpu.VMEM((NT, D, T), f32), pltpu.VMEM((4 * NT, 2 * MP, 256), bf16),
            pltpu.VMEM((NT, NTILE, 64, 128), u32), pltpu.VMEM((NTILE, 64, 128), u32),
            pltpu.VMEM((1024, 256), u32),
            *[pltpu.VMEM((66 * CB, CH), f32)] * 2,
            pltpu.VMEM((2624, 128), f32), pltpu.VMEM((2624, 128), f32),
        ] + [pltpu.VMEM((3840, 128), f32)] * NT + [
            pltpu.SemaphoreType.DMA((NT,)), pltpu.SemaphoreType.DMA((8,)),
            pltpu.SemaphoreType.DMA((3, 3)), pltpu.SemaphoreType.DMA((2, 3)),
            pltpu.SemaphoreType.DMA((4 * NT,)),
        ] + [pltpu.VMEM((2112, 128), f32)] * (2 * NT) + [
            pltpu.VMEM((D, D), bf16), pltpu.VMEM((D, D), bf16),
            pltpu.VMEM((4, D), bf16), pltpu.VMEM((D,), bf16), pltpu.VMEM((D,), bf16)],
        compiler_params=pltpu.CompilerParams(vmem_limit_bytes=124 * 2**20),
    )(A_q[0].T, A_k[0].T, A_v[0].T, A_shift_k.T, A_ssm_k, A_ssm_D,
      B_w1, B_w2, B_w3, B_w4.T, gate_w, np.zeros((16,), np.int32), *_transform_tables())
    return out.T[None]
```

```python
import math
import numpy as np
import jax
import jax.numpy as jnp
from jax import lax
import jax.experimental.pallas as pl
import jax.experimental.pallas.tpu as pltpu

S, D, F = 2048, 576, 4608
CH = 128
NCH = S // CH
f32, bf16, u32 = jnp.float32, jnp.bfloat16, jnp.uint32

T = 512
NT = S // T
FC = 512
NF = F // FC
CS = D // NF
TIES = 12
MP = D // 4
PS, AS, XS = 136, 2 * MP + 8, 72
QT, FR = 6, 32
CB, CI = 32, 64
ORDER = (1, 4, 0, 2, 5, 3, 6)

_C0 = math.sqrt(2.0 / math.pi)
GS = (_C0 * 0.044715) ** (1.0 / 3.0)
GK = _C0 / GS
KAPPA = 0.5 / GS

SA = [{(0, 0): 1, (1, 1): 1}, {(1, 0): 1, (1, 1): 1}, {(0, 0): 1}, {(1, 1): 1},
      {(0, 0): 1, (0, 1): 1}, {(1, 0): 1, (0, 0): -1}, {(0, 1): 1, (1, 1): -1}]
SB = [{(0, 0): 1, (1, 1): 1}, {(0, 0): 1}, {(0, 1): 1, (1, 1): -1}, {(1, 0): 1, (0, 0): -1},
      {(1, 1): 1}, {(0, 0): 1, (0, 1): 1}, {(1, 0): 1, (1, 1): 1}]
SC = np.array([[1, 0, 0, 1], [0, 0, 1, -1], [0, 1, 0, 1], [1, 0, 1, 0], [-1, 1, 0, 0], [0, 0, 0, 1], [1, 0, 0, 0]])


def _single(ps):
    inv = np.rint(np.linalg.inv(SC[list(ps)].astype(np.float64))).astype(int)
    out = {}
    for n, p in enumerate(ps):
        lam = inv[:, n].reshape(2, 2)
        i0, j0 = np.argwhere(lam != 0)[0]
        a, b = lam[:, j0] * lam[i0, j0], lam[i0, :].copy()
        assert (np.outer(a, b) == lam).all()
        if (b <= 0).all():
            a, b = -a, -b
        out[p] = ({i: int(a[i]) for i in range(2) if a[i]}, {j: int(b[j]) for j in range(2) if b[j]})
    return out


_PLAN = {9: (3, [(1, 3, 2, 5), (2, 4, 3, 6), (0, 3, 2, 5)]), 4: (2, []),
         6: (2, [(0, 1, 2, 5), (0, 1, 2, 5)]), 5: (1, [(1, 3, 2, 5), (2, 4, 1, 5), (0, 1, 2, 5)])}


def _level(depth):
    n_pairs, singles = _PLAN[depth]
    terms = [[] for _ in range(7)]
    for t in range(n_pairs):
        kk = (2 * t, 2 * t + 1)
        for p in range(7):
            terms[p].append(({(i, kk[k]): c for (i, k), c in SA[p].items()},
                             {(j, kk[k]): c for (k, j), c in SB[p].items()}))
    for n, ps in enumerate(singles):
        kb = 2 * n_pairs + n
        for p, (a, b) in _single(ps).items():
            terms[p].append(({(i, kb): c for i, c in a.items()}, {(j, kb): c for j, c in b.items()}))
    return terms


def _lin(items):
    acc = None
    for c, v in sorted(items, key=lambda cv: -cv[0]):
        if acc is None:
            acc = v if c > 0 else -v
        else:
            acc = acc + v if c > 0 else acc - v
    return acc


def _deep_operands(blocks, side, levels):
    if levels == 0:
        return [[b[0] for b in blocks]]
    h = len(blocks[0]) // 2
    out = []
    for terms in _level(len(blocks)):
        nxt = [[_lin([(c, blocks[kb][i * h + s]) for (i, kb), c in t[side].items()]) for s in range(h)]
               for t in terms]
        out += _deep_operands(nxt, side, levels - 1)
    return out


def _deep_group(get, side, p1):
    terms = _level(9)[p1]
    nxt = [[_lin([(c, get(kb, i * 2 + s)) for (i, kb), c in t[side].items()]) for s in range(2)] for t in terms]
    return _deep_operands(nxt, side, 1)


class _Sum(dict):
    def __add__(self, other):
        return _Sum({k: v for k in {**self, **other} if (v := self.get(k, 0) + other.get(k, 0))})

    def __neg__(self):
        return _Sum({k: -v for k, v in self.items()})

    def __sub__(self, other):
        return self + -other


_X_TERMS = _deep_operands([[_Sum({(kb, s): 1}) for s in range(4)] for kb in range(9)], 0, 2)
_UP_ORDER = (1, 3, 2, 4, 0, 5, 6)


def _combine7(p):
    return [(p[3] - p[4]) + p[0] + p[6], p[2] + p[4], p[1] + p[3], (p[2] - p[1]) + p[0] + p[5]]


DEPTH = [len(t2) for t1 in _level(9) for t2 in _level(len(t1))]
NPROD = len(DEPTH)
TILE0 = [sum((d + 1) // 2 for d in DEPTH[:p]) for p in range(NPROD + 1)]
NTILE = TILE0[-1]


def _unpack(v):
    return pltpu.bitcast(v, bf16)


def _rows2(w):
    return [pltpu.unpack_elementwise(w, index=i, packed_dtype=bf16, unpacked_dtype=f32) for i in range(2)]


def _join2(even, odd):
    return pltpu.pack_elementwise([even, odd], packed_dtype=bf16)


def _gelu_u(u):
    return u + u * jnp.tanh(u * (u * u + GK))


def _col(row):
    b = jnp.broadcast_to(row, (128, D))
    b = jnp.concatenate([b, jnp.zeros((128, 64), f32)], axis=1)
    return b.T[:D, :]


def _transform_tables():
    def words(x):
        bits = x.astype(bf16).view(np.uint16).astype(np.uint32)
        return bits[:, 0::2] | (bits[:, 1::2] << 16)
    f, lane, m = np.ogrid[:4, :CH, :CH]
    angle = ((4 * m + 1) * (4 * ((lane - 32 * f) % CH) + f) % 2048) * (np.pi / 1024.0)
    fwd = np.concatenate([np.cos(angle), np.sin(angle)], axis=2)
    return words(fwd), words(fwd.transpose(0, 2, 1) / T)


def _kernel(q_hbm, k_hbm, v_hbm, sk_hbm, ssmk_hbm, ssmd_hbm, w1_hbm, w2_hbm, w3_hbm, w4_hbm, gw_hbm,
            zero_hbm, f_hbm, g_hbm, out_hbm,
            zero_ref,
            q_v, k_v, v_v, ssmk_v, w3_v, w4_v, w1t, w2t, cols, fmat, gmat,
            h_v, g_v, x1_v, ga_v, o_v, xa, wb, wa, zb0, zb1, xn0, xn1, pb0, pb1, pb2, pb3,
            sem_q, sem_w, sem_c, sem_f, sem_out, *rest):
    *acc, w1_v, w2_v, sk_ref, ssmd_ref, gw_ref = rest
    pb = (pb0, pb1, pb2, pb3)
    xnb = (xn0, xn1)
    zbs = (zb0, zb1)
    cp_q = [pltpu.make_async_copy(q_hbm.at[:, pl.ds(b * T, T)], q_v.at[b], sem_q.at[b]) for b in range(NT)]
    cp_w1 = pltpu.make_async_copy(w1_hbm, w1_v, sem_w.at[0])
    cp_w2 = pltpu.make_async_copy(w2_hbm, w2_v, sem_w.at[1])
    cp_out = [pltpu.make_async_copy(
        o_v.at[n], out_hbm.at[pl.ds(n % 4 // 2 * 2 * MP, 2 * MP), pl.ds(n // 4 * T + n % 2 * 256, 256)], sem_out.at[n])
        for n in range(4 * NT)]

    def weights(n, chunks, sem):
        src, dst = ((w3_hbm, w3_v), (w4_hbm, w4_v))[n]
        return [pltpu.make_async_copy(src.bitcast(u32).at[:, pl.ds(i * FC, FC)], dst.at[i], sem) for i in chunks]

    def conv_inputs(first, count, group):
        words = pl.ds(first * (CS // 2), count * (CS // 2))
        return [pltpu.make_async_copy(src.bitcast(u32).at[words, :], dst.at[words, :], sem_c.at[group, n])
                for n, (src, dst) in enumerate(((k_hbm, k_v), (v_hbm, v_v), (ssmk_hbm, ssmk_v)))]

    aligned = lambda x, n: x if isinstance(x, int) else pl.multiple_of(x, n)

    def zero(n):
        return pl.multiple_of(zero_ref[n], 64)

    def schedule(pieces, slots):
        total, now, out = sum(w for w, _ in pieces), 0, [[] for _ in range(slots)]
        for w, fn in pieces:
            out[min(slots - 1, int((now + w / 2) * slots / total))].append(fn)
            now += w
        return out

    def both(*plans):
        return [[fn for part in slot for fn in part] for slot in zip(*plans, strict=True)]

    def tied(w, *due):
        step = w.shape[0] // 8 // len(due) * 8
        parts = []
        for j, fns in enumerate(due):
            tie = None
            for fn in fns:
                t = fn()
                if t is not None:
                    t = pltpu.bitcast(t, u32)
                    tie = t if tie is None else tie | t
            top = w[j * step:j * step + 8]
            if tie is not None:
                left = top[:, :128] | (tie & jnp.full((8, 128), zero_ref[0], jnp.int32).astype(u32))
                top = jnp.concatenate([left, top[:, 128:]], axis=1) if w.shape[1] > 128 else left
            parts += [top, w[j * step + 8:(j + 1) * step if j + 1 < len(due) else w.shape[0]]]
        return jnp.concatenate(parts, axis=0)

    def token(w):
        t = w[:8, :128]
        for r in range(8, w.shape[0], 8):
            t = t | w[r:r + 8, :128]
        return t

    def transposed(w):
        w = w.astype(f32)
        w = jnp.concatenate([w, jnp.zeros((D, 64), f32)], axis=1)
        w = jnp.concatenate([w, jnp.zeros((64, D + 64), f32)], axis=0)
        return pltpu.bitcast(w.astype(bf16).T, u32)[:D // 2, :]

    def moments(state, x):
        if not state:
            state.update(pivot=jnp.broadcast_to(x[:1], (8, 128)), s1=None, s2=None)
        for r in range(0, x.shape[0], 8):
            d = x[r:r + 8] - state['pivot']
            state['s1'] = d if state['s1'] is None else state['s1'] + d
            state['s2'] = d * d if state['s2'] is None else state['s2'] + d * d

    def mean_scale(state):
        m = jnp.sum(state['s1'], axis=0, keepdims=True) * (1.0 / D)
        v = jnp.sum(state['s2'], axis=0, keepdims=True) * (1.0 / D) - m * m
        state['mean'] = state['pivot'] + m
        state['scale'] = jnp.broadcast_to(lax.rsqrt(jnp.maximum(v, 0.0) + 1e-5) * GS, (8, 128))
        return state['scale']

    def normalized(state, x):
        return jnp.concatenate([(x[r:r + 8] - state['mean']) * state['scale'] for r in range(0, x.shape[0], 8)], axis=0)

    stats = [{} for _ in range(S // 128)]

    def stats1(n):
        b, s = divmod(n, 4)
        gate = []

        def piece(r):
            x = q_v[b + zero(0), r:r + 48, s * 128:(s + 1) * 128].astype(f32)
            moments(stats[n], x)
            xw = x * cols[5, r:r + 48, :]
            for j in range(0, 48, 8):
                gate[:] = [xw[j:j + 8] + gate[0] if gate else xw[j:j + 8]]
            if r + 48 < D:
                return stats[n]['s2'] + gate[0]
            g = jnp.broadcast_to(jax.nn.sigmoid(jnp.sum(gate[0], axis=0, keepdims=True)), (8, 128))
            g_v[:, n * 128:(n + 1) * 128] = g
            return mean_scale(stats[n]) + g
        return [(42, lambda r=r: piece(r)) for r in range(0, D, 48)]

    def stage1(n, due, sync):
        b, s = divmod(n, 4)
        x = normalized(stats[n], q_v[b + zero(1), :, s * 128:(s + 1) * 128].astype(f32)).astype(bf16)
        sync()
        z = jnp.dot(_unpack(tied(w1t[zero(0), :D // 2, :], *due))[:, :D], x, preferred_element_type=f32)

        def act(r):
            h = _gelu_u(z[r:r + 48])
            h_v[r:r + 48, n * 128:(n + 1) * 128] = h
            return h_v[pl.ds(zero(0), 8), :128]
        return [(36, lambda r=r: act(r)) for r in range(0, D, 48)], []

    def stage2(n, due, sync):
        grp = D // 4
        b, s = divmod(n, 4)
        c0 = n * 128
        w = _unpack(tied(w2t[zero(0), :D // 2, :], *due))[:, :D]
        parts = []
        for gi, k in enumerate((1, -1, 2, -2)):
            rows = slice(gi * grp, (gi + 1) * grp)
            cur = h_v[rows, c0:c0 + 128]
            if k > 0:
                halo = h_v[rows, c0 - 128:c0] if c0 > 0 else jnp.zeros((grp, 128), f32)
                parts.append(pltpu.roll(jnp.concatenate([halo, cur], axis=1), k, 1)[:, 128:])
            else:
                halo = h_v[rows, c0 + 128:c0 + 256] if c0 + 128 < S else jnp.zeros((grp, 128), f32)
                parts.append(pltpu.roll(jnp.concatenate([cur, halo], axis=1), 256 + k, 1)[:, :128])
        z = jnp.dot(w, jnp.concatenate(parts, axis=0).astype(bf16), preferred_element_type=f32)
        c = slice(s * 128, (s + 1) * 128)
        state = {}

        def residual(r):
            x1 = q_v[b + zero(2), r:r + 48, c].astype(f32) + z[r:r + 48]
            x1_v[b, r:r + 48, c] = x1
            moments(state, x1)
            return state['s2'] if r + 48 < D else mean_scale(state)

        def norm(r):
            row = (s * 9 + r // 64) * XS
            xnb[b % 2][row:row + 64, :] = normalized(state, x1_v[b + zero(0), r:r + 64, c])
            return xnb[b % 2][pl.ds(zero(0), 8), :]
        return ([(40, lambda r=r: residual(r)) for r in range(0, D, 48)],
                [(24, lambda r=r: norm(r)) for r in range(0, D, 64)])

    def x_operands(b):
        def piece(p, n):
            pair = [_lin([(c, xnb[b % 2][pl.ds(zero(8 + p % 7) + (s * 9 + kb) * XS, 64), :])
                          for (kb, s), c in terms.items()]) for terms in _X_TERMS[p][2 * n:2 * n + 2]]
            if len(pair) == 1:
                pair.append(jnp.zeros((64, 128), f32))
            w = pltpu.bitcast(jnp.concatenate(pair, axis=0).astype(bf16).T, u32)
            xa[b, TILE0[p] + n] = w
            return w[56:]

        return [(4 + sum(map(len, _X_TERMS[p][2 * n:2 * n + 2])), lambda p=p, n=n: piece(p, n))
                for p in range(NPROD) for n in range(TILE0[p + 1] - TILE0[p])]

    def w3_operands(i):
        groups = {}

        def piece(p, n):
            p1, p2 = divmod(p, 7)
            if p1 not in groups:
                ii = i + zero(8 + p1)
                words = lambda kb, s: _rows2(w3_v[ii, kb * 32:(kb + 1) * 32, s * 128:(s + 1) * 128])
                groups[p1] = [_deep_group(lambda kb, s: words(kb, s)[h], 1, p1) for h in range(2)]
            w = _join2(groups[p1][0][p2][n], groups[p1][1][p2][n])
            wb[TILE0[p] + n // 2, (n % 2) * 32:(n % 2) * 32 + 32, :] = w
            return token(w)

        return [(17, lambda p=p, n=n: piece(p, n)) for p in range(NPROD) for n in range(DEPTH[p])]

    def w4_operands(i):
        def piece(p, r):
            words = [(c, _rows2(w4_v[i + zero(8 + p), m * MP + r:m * MP + r + 48, k * 256:(k + 1) * 256]))
                     for (m, k), c in SA[p].items()]
            w = _join2(*[_lin([(c, w[h]) for c, w in words]) for h in range(2)])
            wa[p * MP + r:p * MP + r + 48, :] = w
            return token(w[:, :128] | w[:, 128:])
        return [(40, lambda p=p, r=r: piece(p, r)) for p in ORDER if len(SA[p]) > 1 for r in range(0, MP, 48)]

    def long_conv(i):
        kv, spec = {}, {}
        words = lambda r: pl.ds(aligned(i * (CS // 2), CS // 2) + r // 2, 8)
        lane = lambda n: lax.broadcasted_iota(jnp.int32, (n, 128), 1)
        zrow = lambda r, sig, n, c, h: ((r % CB // 8) * 65 + sig * 32 + n * 8 + c * 2 + h) * 8

        def quarters(p):
            ln = lane(p[0].shape[0])
            even, low, mid = (ln & 32) == 0, ln < 64, ((ln + 32) & 64) != 0
            r0, r1 = jnp.where(even, p[0], p[1]), jnp.where(even, p[2], p[3])
            r2, r3 = jnp.where(even, p[1], p[0]), jnp.where(even, p[3], p[2])
            return [jnp.where(low, r0, r1), jnp.where(mid, r2, r3), jnp.where(low, r1, r0), jnp.where(mid, r3, r2)]

        def to_phases(v):
            ln = lane(v[0].shape[0])
            return quarters([jnp.take_along_axis(v[a], 4 * (ln & 31) + (((ln >> 5) - a) & 3), axis=1) for a in range(4)])

        def from_phases(x):
            ln = lane(x[0].shape[0])
            return [jnp.take_along_axis(p, 32 * ((ln + a) & 3) + (ln >> 2), axis=1) for a, p in enumerate(quarters(x))]

        def short_conv(r, a):
            cur = k_v[words(r), a * CH:(a + 1) * CH]
            old = k_v[words(r), (a - 1) * CH:a * CH] if a else jnp.zeros((8, CH), u32)
            taps = [_rows2(cur)] + [_rows2(jnp.where(lane(8) >= j, pltpu.roll(cur, j, 1), pltpu.roll(old, j, 1)))
                                    for j in range(1, 4)]
            vv = _rows2(v_v[words(r), a * CH:(a + 1) * CH])
            x = []
            for h in range(2):
                rows = pl.ds(aligned(i * CS, CS) + r + h, 8, stride=2)
                ks = taps[0][h] * cols[0, rows, :]
                for j in range(1, 4):
                    ks = ks + taps[j][h] * cols[j, rows, :]
                x.append(ks * vv[h])
            kv[r, a] = _join2(*x)
            return kv[r, a]

        def spectra(r0, sig):
            rs = range(r0, r0 + CB, 16)
            if sig == 0:
                get = lambda r, a: ssmk_v[words(r), a * CH:(a + 1) * CH]
            else:
                get = lambda r, a: kv[r, a]
            ph = {(c, r): to_phases([get(r, 4 * c + a) for a in range(4)]) for c in range(4) for r in rs}
            zb = zbs[r0 // CB]
            for odd in range(2):
                z = [jnp.dot(_unpack(jnp.concatenate([ph[c, r][f] for c in range(4) for r in rs], axis=0)),
                             _unpack(fmat[f]), preferred_element_type=f32) for f in (odd, odd + 2)]
                for n, v in enumerate((z[0] + z[1], z[0] - z[1])):
                    for c in range(4):
                        for r in range(0, CB, 8):
                            for h in range(2):
                                row = zrow(r, sig, 2 * odd + n, c, h)
                                zb[row:row + 8, :] = v[c * CB + r:c * CB + r + 8, h * CH:(h + 1) * CH]

        def loader(r):
            zb, r16 = zbs[r // CB], r // 16 * 16

            def load(sig, n, c, h):
                return zb[pl.ds(zero(0) + zrow(r, sig, n, c, h), 8), :]
            return load

        ext = {}

        def spectrum(r, sig, l, c):
            if (r, sig, l, c) not in ext:
                load = loader(r)
                ar, ai = load(sig, l % 2, c, 0), load(sig, l % 2, c, 1)
                br, bi = load(sig, 2 + l % 2, c, 0), load(sig, 2 + l % 2, c, 1)
                ext[r, sig, l, c] = [(ar + br, ai + bi), (ar - bi, ai + br), (ar - br, ai - bi), (ar + bi, ai - br)][l]
            return ext[r, sig, l, c]

        def window(r, l, c):
            if (r, 2, l, c) not in ext:
                kr, ki = spectrum(r, 0, l, c)
                if c:
                    pr, pi = spectrum(r, 0, l, c - 1)
                    ext[r, 2, l, c] = (kr + pi, ki - pr)
                else:
                    ext[r, 2, l, c] = (kr + cols[4, pl.ds(aligned(i * CS, CS) + r, 8), :], ki)
            return ext[r, 2, l, c]

        def product(r, l, c):
            yr = yi = None
            for j in range(c + 1):
                (kr, ki), (ur, ui) = window(r, l, j), spectrum(r, 1, l, c - j)
                tr, ti = kr * ur - ki * ui, kr * ui + ki * ur
                yr, yi = (tr, ti) if j == 0 else (yr + tr, yi + ti)
            ext[r, 3, l, c] = (yr, yi)
            if l < 2:
                return yr + yi
            (ar, ai), (br, bi) = ext[r, 3, l - 2, c], (yr, yi)
            ext[r, 4, l - 2, c] = (ar + br, ai + bi, ar - br, ai - bi)
            if l == 2:
                return ext[r, 4, 0, c][2] + ext[r, 4, 0, c][3]
            (s0r, s0i, d0r, d0i), (s1r, s1i, d1r, d1i) = ext[r, 4, 0, c], ext[r, 4, 1, c]
            for f, v in enumerate(((s0r + s1r, s0i + s1i), (d0r + d1i, d0i - d1r),
                                   (s0r - s1r, s0i - s1i), (d0r - d1i, d0i + d1r))):
                spec[f, c, r] = jnp.concatenate(v, axis=1)
            return spec[3, c, r][:, :CH] + spec[3, c, r][:, CH:]

        def inverse(r0):
            y = [jnp.dot(jnp.concatenate([spec[f, c, r] for c in range(4) for r in range(r0, r0 + CI, 8)],
                                         axis=0).astype(bf16),
                         _unpack(gmat[f]), preferred_element_type=f32) for f in range(4)]
            rows = pl.ds(aligned(i * CS, CS) + r0, CI)
            for b in range(NT):
                yb = jnp.concatenate(from_phases([y[f][b * CI:(b + 1) * CI, :] for f in range(4)]), axis=1)
                g = g_v[0:1, b * T:(b + 1) * T]
                ga_v[b, rows, :] = g * (q_v[b, rows, :].astype(f32) * yb) + (1.0 - g) * x1_v[b, rows, :]

        def inverse_all():
            for r in range(0, CS, CI):
                inverse(r)

        return ([[(30, lambda r=r, a=a: short_conv(r, a)) for a in range(NCH)] for r in range(0, CS, 16)],
                [[(0, lambda r=r: spectra(r, 0))] for r in range(0, CS, CB)],
                [[(0, lambda r=r: spectra(r, 1))] for r in range(0, CS, CB)],
                [[(8 * c + 12, lambda r=r + h, l=l, c=c: product(r, l, c))
                  for h in (0, 8) for l in (0, 2, 1, 3) for c in range(4)] for r in range(0, CS, 16)],
                inverse_all)

    def up(i, t, p1, due):
        pv = {}
        for p2 in _UP_ORDER:
            p = p1 * 7 + p2
            n = TILE0[p + 1] - TILE0[p]
            a = jnp.concatenate([_unpack(tied(xa[zero(5) + t, TILE0[p] + j], next(due))) for j in range(n)], axis=1)
            bt = [_unpack(wb[zero(1 + t) + TILE0[p] + j, :min(64, DEPTH[p] * 32 - 64 * j), :]) for j in range(n)]
            pv[p2] = jnp.dot(a[:, :DEPTH[p] * 64], jnp.concatenate(bt, axis=0), preferred_element_type=f32)
        for q, c in enumerate(_combine7(pv)):
            pb[t][(q * 7 + p1) * PS:(q * 7 + p1) * PS + 128, :] = c

    def down(i, t, due):
        hid = {}

        def hidden(k, s):
            if (k, s) not in hid:
                q, q2 = (s // 2) * 2 + k // 2, (s % 2) * 2 + k % 2
                hid[k, s] = _gelu_u(_lin([(SC[p1, q], pb[t][pl.ds(zero(0) + (q2 * 7 + p1) * PS, 128), :])
                                          for p1 in range(7) if SC[p1, q]]))
            return hid[k, s]

        for p in ORDER:
            if len(SA[p]) > 1:
                w = wa[pl.ds(zero(1 + t) + p * MP, MP), :]
            else:
                (m, k), = SA[p]
                w = w4_v[i + zero(1 + t), m * MP:(m + 1) * MP, k * 256:(k + 1) * 256]
            hv = jnp.concatenate([jnp.concatenate(
                [_lin([(c, hidden(2 * k + h, 2 * j + s)) for (k, j), c in SB[p].items()]) for h in range(2)], axis=1)
                for s in range(2)], axis=0)
            y = lax.dot_general(_unpack(tied(w, *[next(due) for _ in range(QT)])), hv.astype(bf16),
                                (((1,), (1,)), ((), ())), preferred_element_type=f32)
            for s in range(2):
                acc[2 * t + s][p * AS:p * AS + 2 * MP, :] += y[:, s * 128:(s + 1) * 128]

    def finish(t, q):
        def piece(r):
            rows = slice(q // 2 * 2 * MP + r, q // 2 * 2 * MP + r + FR)
            c0 = q % 2 * 256
            h2 = jnp.concatenate([_lin([(SC[p, q], acc[2 * t + s][pl.ds(zero(0) + p * AS + r, FR), :])
                                        for p in range(7) if SC[p, q]]) for s in range(2)], axis=1)
            og = (1.0 - g_v[0:1, t * T + c0:t * T + c0 + 256]) * KAPPA
            out = ga_v[t, rows, c0:c0 + 256] + og * h2
            o_v[4 * t + q, r:r + FR, :] = out.astype(bf16)
            return out[FR - 8:, :128] + out[FR - 16:FR - 8, 128:]
        return [(1, lambda r=r: piece(r)) for r in range(0, 2 * MP, FR)]

    def send(*blocks):
        def start():
            for n in blocks:
                cp_out[n].start()
        return [(0, start)]

    idle = lambda n: [[]] * n

    def ups(i, t, due):
        due = iter(due)
        for p1 in range(7):
            up(i, t, p1, due)

    def transforms(i):
        kv, filt, data, _, _ = long_conv(i)
        return filt[0] + kv[0] + filt[1] + kv[1] + kv[2][:4] + data[0] + kv[2][4:] + kv[3], data[1]

    def chunk(i, last=False):
        _, _, _, mac, inverse = long_conv(i)
        v = w4_operands(i)
        nm = 16 if last else 24
        mac = mac[0] + mac[1] + mac[2] + mac[3]
        due = schedule(mac[:nm] + v + mac[nm:], 3 * NTILE)
        for t in range(1, NT):
            ups(i, t, due[(t - 1) * NTILE:t * NTILE])
        if last:
            inverse()
            fs, lag = 8, 4
            whole = lambda t: finish(t, 1) + finish(t, 3) + finish(t, 2) + finish(t, 0)
            down(i, 0, iter(idle(7 * QT)))
            down(i, 1, iter(idle(fs) + schedule(whole(0) + send(0, 1, 2, 3), 7 * QT - fs)))
            down(i, 2, iter(idle(fs) + schedule(whole(1) + send(4, 5, 6, 7), 7 * QT - fs)))
            down(i, 3, iter(idle(fs) + schedule(whole(2) + send(8, 9, 10, 11), 4 * QT + lag - fs)
                            + schedule(finish(3, 1), QT) + schedule(finish(3, 3) + send(13, 15), QT)
                            + schedule(finish(3, 2), QT - lag)))
            for _, fn in send(14) + finish(3, 0) + send(12):
                fn()
            return
        q0, q1 = 6, 150
        due = iter(idle(q0) + schedule(w3_operands(i + 1), q1 - q0) + idle(28 * QT - q1))
        for t in range(NT):
            down(i, t, due)
        early, late = transforms(i + 1)
        te = 50
        due = schedule(early, te) + idle(8) + [[late[0][1]]] + idle(NTILE)
        due[35] = due[35] + [inverse]
        ups(i + 1, 0, due)

    head = [cp_w1, cp_q[0]]
    small = [pltpu.make_async_copy(src, dst, sem_w.at[4 + n]) for n, (src, dst) in enumerate(
        ((zero_hbm, zero_ref), (sk_hbm, sk_ref), (ssmd_hbm, ssmd_ref), (gw_hbm, gw_ref)))]
    for cp in small + head:
        cp.start()
    for ref in acc[:4]:
        for p in range(7):
            ref[p * AS:p * AS + 2 * MP, :] = jnp.zeros((2 * MP, 128), f32)
    for cp in small:
        cp.wait()

    sk = sk_ref[...].astype(f32)
    for j in range(4):
        cols[j] = _col(sk[j:j + 1, :])
    cols[4] = _col(ssmd_ref[...].astype(f32).reshape(1, D))
    cols[5] = _col(gw_ref[...].astype(f32).reshape(1, D))
    for ref in acc[4:]:
        for p in range(7):
            ref[p * AS:p * AS + 2 * MP, :] = jnp.zeros((2 * MP, 128), f32)

    n1 = 13
    order = ([(1, n) for n in range(n1)] + [(2, n) for n in range(4)] + [(1, n) for n in range(n1, 16)]
             + [(2, n) for n in range(4, 16)])
    times = [n / TIES for n in range(len(order) * TIES)] + [len(order) + n * 32 / 720 for n in range(NTILE)]
    due = [[] for _ in times]

    def place(pieces, d0, d1):
        slots = [n for n, d in enumerate(times) if d0 <= d < d1]
        for slot, fns in zip(slots, schedule(pieces, len(slots))):
            due[slot] += fns

    def w2_part(j):
        n = min(128, D - 128 * j)
        w = w2_v[:, 128 * j:128 * j + n].astype(f32) * KAPPA
        w = jnp.concatenate([w, jnp.zeros((64, n), f32)], axis=0)
        if n < 128:
            w = jnp.concatenate([w, jnp.zeros((D + 64, 128 - n), f32)], axis=1)
        w = pltpu.bitcast(w.astype(bf16).T, u32)[:n // 2]
        w2t[0, 64 * j:64 * j + n // 2, :] = w
        return w[:8, 512:]

    ready = 0
    place([(1, lambda j=j: w2_part(j)) for j in range(5)], 11.2, n1 - 0.5)
    place(w3_operands(0), 13, 19)
    early, late = transforms(0)
    place([e for e in early if e[0]], 22, 27)
    place([(1, e[1]) for e in early if not e[0]], len(order) + 1.4, 99)
    for d, (stage, n) in enumerate(order):
        if stage == 1 and d:
            place(stats1(n), d - 1, d - 0.6)

    for cp in head:
        cp.wait()
    second = [cp_q[1], cp_q[2], pltpu.make_async_copy(f_hbm, fmat, sem_w.at[2])]
    third = [cp_q[3], cp_w2] + weights(0, [0], sem_f.at[0, 0]) + conv_inputs(0, 1, 0)
    fourth = ([pltpu.make_async_copy(g_hbm, gmat, sem_w.at[3])] + weights(0, [1, 2], sem_f.at[0, 1])
              + weights(1, [0, 1], sem_f.at[1, 1]) + conv_inputs(1, 2, 1))
    fifth = weights(0, range(3, NF), sem_f.at[0, 2]) + weights(1, range(2, NF), sem_f.at[1, 2]) + conv_inputs(3, NF - 3, 2)
    for cp in second:
        cp.start()
    w1t[0, :D // 2, :] = transposed(w1_v[...])
    for _, fn in stats1(0):
        fn()

    def sync(d):
        for cp in {3: second, 11: third}.get(d, []):
            cp.wait()
        if d == 3:
            for cp in third:
                cp.start()
        if d == 11:
            @pl.loop(0, 1 + zero_ref[0])
            def _(_):
                for cp in fourth:
                    cp.start()

    for d, (stage, n) in enumerate(order):
        one, two = (stage1, stage2)[stage - 1](n, due[d * TIES:(d + 1) * TIES], lambda: sync(d))
        lag, lag2 = 1.3, 1.2
        if d >= 31:
            lag, lag2 = 1.2, 0.6
        place(one, d + lag, d + lag + min(1, lag2))
        if two:
            place(two, d + lag + lag2, d + lag + lag2 + min(1, lag2))
            ready = max(ready, d + lag + lag2 + min(1, lag2))
        if stage == 2 and n % 4 == 3:
            place(x_operands(n // 4), ready, ready + 3)
    due[-8] += [late[0][1]]
    ups(0, 0, due[len(order) * TIES:])
    for cp in fourth:
        cp.wait()
    for cp in fifth:
        cp.start()

    def arrived():
        for cp in fifth:
            cp.wait()

    @pl.loop(0, NF - 1)
    def _(i):
        pl.when(i == 2)(arrived)
        chunk(i)

    chunk(NF - 1, last=True)
    for cp in cp_out:
        cp.wait()


@jax.jit
def pallas_gated_mix__ssm_conv_h3__mixer_s_mlp__prompt_kernel(A_q, A_k, A_v, A_shift_k, A_ssm_k, A_ssm_D, B_x, B_w1, B_w2, B_w3, B_w4, gate_w):
    del B_x
    hbm = pl.BlockSpec(memory_space=pl.ANY)
    out = pl.pallas_call(
        _kernel,
        out_shape=jax.ShapeDtypeStruct((D, S), bf16),
        in_specs=[hbm] * 14,
        out_specs=hbm,
        scratch_shapes=[
            pltpu.SMEM((16,), jnp.int32),
            pltpu.VMEM((NT, D, T), bf16),
            *[pltpu.VMEM((D // 2, S), u32)] * 3,
            pltpu.VMEM((NF, D // 2, FC), u32), pltpu.VMEM((NF, D // 2, FC), u32),
            pltpu.VMEM((1, 320, 640), u32), pltpu.VMEM((1, 320, 640), u32),
            pltpu.VMEM((6, D, 128), f32),
            pltpu.VMEM((4, CH // 2, 2 * CH), u32), pltpu.VMEM((4, CH, CH), u32),
            pltpu.VMEM((D, S), f32), pltpu.VMEM((8, S), f32),
            pltpu.VMEM((NT, D, T), f32), pltpu.VMEM((NT, D, T), f32), pltpu.VMEM((4 * NT, 2 * MP, 256), bf16),
            pltpu.VMEM((NT, NTILE, 64, 128), u32), pltpu.VMEM((NTILE, 64, 128), u32),
            pltpu.VMEM((1024, 256), u32),
            *[pltpu.VMEM((66 * CB, CH), f32)] * 2,
            pltpu.VMEM((2624, 128), f32), pltpu.VMEM((2624, 128), f32),
        ] + [pltpu.VMEM((3840, 128), f32)] * NT + [
            pltpu.SemaphoreType.DMA((NT,)), pltpu.SemaphoreType.DMA((8,)),
            pltpu.SemaphoreType.DMA((3, 3)), pltpu.SemaphoreType.DMA((2, 3)),
            pltpu.SemaphoreType.DMA((4 * NT,)),
        ] + [pltpu.VMEM((2112, 128), f32)] * (2 * NT) + [
            pltpu.VMEM((D, D), bf16), pltpu.VMEM((D, D), bf16),
            pltpu.VMEM((4, D), bf16), pltpu.VMEM((D,), bf16), pltpu.VMEM((D,), bf16)],
        compiler_params=pltpu.CompilerParams(vmem_limit_bytes=124 * 2**20),
    )(A_q[0].T, A_k[0].T, A_v[0].T, A_shift_k.T, A_ssm_k, A_ssm_D,
      B_w1, B_w2, B_w3, B_w4.T, gate_w, np.zeros((16,), np.int32), *_transform_tables())
    return out.T[None]
```
